```python
import jax
import jax.numpy as jnp

def _softmax(x, axis=-1):
    return jax.nn.softmax(x, axis=axis)
def _gelu(x):
    return jax.nn.gelu(x, approximate=True)
def _silu(x):
    return jax.nn.silu(x)
def _sigmoid(x):
    return jax.nn.sigmoid(x)
def _layernorm(x, axis=-1, eps=1e-5):
    m = jnp.mean(x, axis=axis, keepdims=True)
    v = jnp.var(x, axis=axis, keepdims=True)
    return (x - m) / jnp.sqrt(v + eps)
def _scatter_add(tgt, idx, src, axis=0):
    return tgt.at[idx].add(src)
def _segment_sum(src, seg, n):
    return jax.ops.segment_sum(src, seg, n)
class _Rng:
    def __init__(self, key):
        self._k = key
    def _next(self):
        self._k, sub = jax.random.split(self._k)
        return sub
    def normal(self, shape):
        return jax.random.normal(self._next(), shape, dtype=jnp.bfloat16)
    def randint(self, lo, hi, shape):
        return jax.random.randint(self._next(), shape, lo, hi, dtype=jnp.int32)
    def uniform(self, shape, lo=0.0, hi=1.0):
        return jax.random.uniform(self._next(), shape, jnp.bfloat16, lo, hi)
    def permutation(self, n):
        return jax.random.permutation(self._next(), n)


kernel_name = 'concat_heads__ssm_conv_h3__sliding_local_dilated__prompt'

def setup_inputs():
    _rng = _Rng(jax.random.key(int.from_bytes(__import__("os").urandom(4), "little")))
    _w = (lambda a: (lambda t: t.astype(jnp.bfloat16) if jnp.issubdtype(t.dtype, jnp.floating) else t)(jnp.asarray(a)))
    def _A_setup():
        B, S, D = 1, 2048, 1024
        ks = 4
        return {
            "q": _w((lambda *s: _rng.normal(s) * 0.05)(B, S, D)),
            "k": _w((lambda *s: _rng.normal(s) * 0.05)(B, S, D)),
            "v": _w((lambda *s: _rng.normal(s) * 0.05)(B, S, D)),
            "shift_k": _w((lambda *s: _rng.normal(s) * 0.05)(D, ks) * 0.5),
            "ssm_k": _w((lambda *s: _rng.normal(s) * 0.05)(D, S) * (1.0 / S ** 0.5)),
            "ssm_D": _w((lambda *s: _rng.normal(s) * 0.05)(D)),
        }
    _A_in = _A_setup()

    def _B_setup():
        B, S, D = 1, 2048, 1024
        return {
            "x": _w((lambda *s: _rng.normal(s) * 0.05)(B, S, D)),
            "wqkv": _w((lambda *s: _rng.normal(s) * 0.05)(D, 3 * D)),
            "wo": _w((lambda *s: _rng.normal(s) * 0.05)(D, D)),
        }
    _B_in = _B_setup()

    return {
        "A_q": _A_in["q"],
        "A_k": _A_in["k"],
        "A_v": _A_in["v"],
        "A_shift_k": _A_in["shift_k"],
        "A_ssm_k": _A_in["ssm_k"],
        "A_ssm_D": _A_in["ssm_D"],
        "B_x": _B_in["x"],
        "B_wqkv": _B_in["wqkv"],
        "B_wo": _B_in["wo"],
    }

def reference(A_q, A_k, A_v, A_shift_k, A_ssm_k, A_ssm_D, B_x, B_wqkv, B_wo):
    def _A_ref(q, k, v, shift_k, ssm_k, ssm_D):
        B, S, D = q.shape
        ks = shift_k.shape[-1]
        k_pad = jnp.pad(k, ((0, 0), (ks - 1, 0), (0, 0)))
        k_shift = jnp.zeros_like(k)
        for t in range(ks):
            k_shift = k_shift + k_pad[:, t:t + S, :] * shift_k[:, ks - 1 - t][None, None, :]
        kv = k_shift * v
        L = 2 * S
        kv_pad = jnp.pad(kv, ((0, 0), (0, S), (0, 0)))
        kf_pad = jnp.pad(ssm_k, ((0, 0), (0, S)))
        kv_f = (lambda x, axes=(-2,-1): jnp.fft.rfft2(x.astype(jnp.float32), axes=axes))(kv_pad[:, None, :, :], axes=(1, 2))
        kf_f = (lambda x, axes=(-2,-1): jnp.fft.rfft2(x.astype(jnp.float32), axes=axes))(kf_pad[:, None, :], axes=(1, 2))
        kf_f = (lambda x, *d: x.transpose(*d))(kf_f, 1, 2, 0)
        y_f = kv_f * kf_f[None, :, :, :]
        y = (lambda x, s, axes=(-2,-1): jnp.fft.irfft2(x, s=s, axes=axes).astype(jnp.bfloat16))(y_f, (1, L), axes=(1, 2))[:, 0, :S, :]
        y = y + kv * ssm_D[None, None, :]
        return q * y

    def _B_ref(x, wqkv, wo):
        B, S, D = x.shape
        H = 32; Dh = D // H
        W, dil = 8, 2
        qkv = (lambda x, *d: x.transpose(*d))((x @ wqkv).reshape(B, S, 3, H, Dh), 2, 0, 3, 1, 4)
        q, k, v = qkv[0], qkv[1], qkv[2]
        scale = Dh ** -0.5
        pos = jnp.arange(S)
        off = jnp.arange(W) * dil
        idx = pos[:, None] - off[None, :]
        mask = idx >= 0
        idx_c = jnp.where(mask, idx, 0).reshape(-1)
        kg = k[:, :, idx_c, :].reshape(B, H, S, W, Dh)
        vg = v[:, :, idx_c, :].reshape(B, H, S, W, Dh)
        logits = jnp.einsum("bhsd,bhswd->bhsw", q, kg) * scale
        logits = jnp.where(mask[None, None, :, :], logits, -1e9)
        attn = _softmax(logits, axis=-1)
        o = jnp.einsum("bhsw,bhswd->bhsd", attn, vg)
        return (lambda x, *d: x.transpose(*d))(o, 0, 2, 1, 3).reshape(B, S, D) @ wo

    a = _A_ref(A_q, A_k, A_v, A_shift_k, A_ssm_k, A_ssm_D)
    b = _B_ref(B_x, B_wqkv, B_wo)
    return jnp.concatenate([a, b], axis=-1)
```

```python
import functools

import numpy as np
import jax
import jax.numpy as jnp
import jax.experimental.pallas as pl
import jax.experimental.pallas.tpu as pltpu

S = 2048
D = 1024
NH = 32
DH = 32
WIN = 8
DIL = 2
NSTEP = 8
RB = S // NSTEP
SUB = 128
HALO = 16
NBLK = 16
F32 = jnp.float32
BF16 = jnp.bfloat16
U32 = jnp.uint32
NT = (((1,), (1,)), ((), ()))


def _constants():
    forder = np.concatenate([np.arange(0, 64, 2), np.arange(1, 64, 2)])
    theta = np.pi * (2 * forder + 1) / 256.0
    j = np.arange(128)
    ang = theta[:, None] * j[None, :]
    sgn = np.where(j % 2 == 0, 1.0, -1.0)[None, :]
    a_re, a_im = np.cos(ang), -np.sin(ang)
    b_re, b_im = a_re * sgn, a_im * sgn
    fwd = np.zeros((256, 128))
    for g in range(8):
        sl = slice(8 * g, 8 * g + 8)
        fwd[32 * g + 0:32 * g + 8] = a_re[sl]
        fwd[32 * g + 8:32 * g + 16] = a_im[sl]
        fwd[32 * g + 16:32 * g + 24] = b_re[sl]
        fwd[32 * g + 24:32 * g + 32] = b_im[sl]
    col = np.zeros(128, np.int64)
    for r in range(8):
        col[16 * r:16 * r + 8] = 16 * r + 2 * np.arange(8)
        col[16 * r + 8:16 * r + 16] = 16 * r + 2 * np.arange(8) + 1
    fwd_u = fwd[:, col]
    inv = np.zeros((2, 64, 128))
    s = np.arange(64)
    for p in range(2):
        a = (2 * s + p)[:, None] * theta[None, :]
        for g in range(8):
            sl = slice(8 * g, 8 * g + 8)
            inv[p, :, 16 * g:16 * g + 8] = np.cos(a[:, sl]) / 128.0
            inv[p, :, 16 * g + 8:16 * g + 16] = -np.sin(a[:, sl]) / 128.0
    perm = np.zeros((2, 128, 128))
    for jj in range(16):
        for r in range(8):
            hh = r % 4
            perm[0, 8 * jj + r, hh * 32 + 2 * jj + (r // 4)] = 1.0
            perm[1, 8 * jj + r, hh * 32 + 2 * jj + 1 - (r // 4)] = 1.0
    fw = np.stack([fwd, fwd_u])
    return (jnp.asarray(fw, BF16), jnp.asarray(inv, BF16), jnp.asarray(perm, BF16))


def _lo(w):
    return pltpu.bitcast(w << 16, F32)


def _hi(w):
    return pltpu.bitcast(w & jnp.uint32(0xFFFF0000), F32)


def _kernel(q_ref, k_ref, v_ref, par_ref, h_ref, x_ref, fw_ref, inv_ref, perm_ref,
            wqkv_hbm, wo_hbm, out_hbm,
            wraw, woraw, wt, wop, qs, ks, vs, ob, ub, uf, uh, hh, eo, outa, outb,
            wsem, osem):
    step = pl.program_id(0)
    slot = step % 2

    def outa_copy(sl, st):
        return pltpu.make_async_copy(
            outa.at[sl], out_hbm.at[:, pl.ds(pl.multiple_of(st * 128, 128), 128)], osem.at[0, sl])

    def outb_copy(sl, st):
        return pltpu.make_async_copy(
            outb.at[sl], out_hbm.at[pl.ds(pl.multiple_of(st * RB, RB), RB), pl.ds(D, D)],
            osem.at[1, sl])

    @pl.when(step == 0)
    def _prologue():
        cps = [pltpu.make_async_copy(wqkv_hbm.at[:, pl.ds(p * D, D)], wraw.at[p], wsem.at[p])
               for p in range(3)]
        cpo = [pltpu.make_async_copy(wo_hbm.at[:, pl.ds(128 * c, 128)], woraw.at[c],
                                     wsem.at[3 + c]) for c in range(8)]
        for cp in cps + cpo:
            cp.start()
        ks[:, pl.ds(0, HALO), :] = jnp.zeros((8, HALO, 128), F32)
        vs[:, pl.ds(0, HALO), :] = jnp.zeros((8, HALO, 128), F32)
        low = jax.lax.broadcasted_iota(jnp.int32, (16, 8, 128), 1) < 4
        for p in range(3):
            cps[p].wait()

            def body(kt, carry, p=p):
                k0 = pl.multiple_of(kt * 128, 128)
                for h4 in range(2):
                    ev, od = [], []
                    for h3 in range(2):
                        t = h4 * 4 + h3 * 2
                        s0 = jax.lax.dot_general(
                            perm_ref[0], wraw[p, pl.ds(k0, 128), pl.ds(128 * t, 128)], NT,
                            preferred_element_type=F32).reshape(16, 8, 128)
                        s1 = jax.lax.dot_general(
                            perm_ref[1], wraw[p, pl.ds(k0, 128), pl.ds(128 * (t + 1), 128)], NT,
                            preferred_element_type=F32).reshape(16, 8, 128)
                        ev.append(jnp.where(low, s0, s1))
                        od.append(pltpu.roll(jnp.where(low, s1, s0), 4, 1))
                    for jj in range(16):
                        for par, src in ((0, ev), (1, od)):
                            row = p * D + (2 * jj + par) * 32 + h4 * 16
                            blk = jnp.concatenate([src[0][jj], src[1][jj]], axis=0)
                            wt[kt, pl.ds(row, 16), :] = blk.astype(BF16)
                return carry

            jax.lax.fori_loop(0, 8, body, 0)
        for cp in cpo:
            cp.wait()
        wo32 = woraw.bitcast(U32)
        wop32 = wop.bitcast(U32)

        def body2(c, carry):
            for dd in range(16):
                for h4 in range(2):
                    a = wo32[c, pl.ds(h4 * 256 + dd, 8, stride=32), :]
                    b = wo32[c, pl.ds(h4 * 256 + 16 + dd, 8, stride=32), :]
                    wop32[c, pl.ds((2 * dd) * 16 + h4 * 8, 8), :] = (
                        (a & jnp.uint32(0xFFFF)) | (b << 16))
                    wop32[c, pl.ds((2 * dd + 1) * 16 + h4 * 8, 8), :] = (
                        (a >> 16) | (b & jnp.uint32(0xFFFF0000)))
            return carry

        jax.lax.fori_loop(0, 8, body2, 0)

    @pl.when(step >= 2)
    def _():
        outa_copy(slot, step - 2).wait()
        outb_copy(slot, step - 2).wait()

    k32 = k_ref.bitcast(U32)
    v32 = v_ref.bitcast(U32)
    q32 = q_ref.bitcast(U32)
    par = par_ref[...].astype(F32)
    taps = [jnp.broadcast_to(par[j:j + 1, :], (8, 128)) for j in range(5)]
    row8 = jax.lax.broadcasted_iota(jnp.int32, (8, 128), 0)

    def a_fwd_h(m):
        hh[m] = jax.lax.dot_general(fw_ref[0], h_ref[:, pl.ds(128 * m, 128)], NT,
                                    preferred_element_type=F32)

    def a_prep(i):
        for r in range(8 * i, 8 * i + 8):
            w0 = k32[pl.ds(8 * r, 8), :]
            if r == 0:
                w1 = jnp.where(row8 < 1, jnp.uint32(0), pltpu.roll(w0, 1, 0))
                w2 = jnp.where(row8 < 2, jnp.uint32(0), pltpu.roll(w0, 2, 0))
            else:
                w1 = k32[pl.ds(8 * r - 1, 8), :]
                w2 = k32[pl.ds(8 * r - 2, 8), :]
            e0, o0, e1, o1, o2 = _lo(w0), _hi(w0), _lo(w1), _hi(w1), _hi(w2)
            kse = taps[0] * e0 + taps[1] * o1 + taps[2] * e1 + taps[3] * o2
            kso = taps[0] * o0 + taps[1] * e0 + taps[2] * o1 + taps[3] * e1
            wv = v32[pl.ds(8 * r, 8), :]
            ue = kse * _lo(wv)
            uo = kso * _hi(wv)
            ub[pl.ds(16 * r, 16), :] = jnp.concatenate([ue, uo], axis=0).astype(BF16)
            uf[0, pl.ds(8 * r, 8), :] = ue * taps[4]
            uf[1, pl.ds(8 * r, 8), :] = uo * taps[4]

    def a_fwd_u(i):
        uh[i] = jnp.dot(fw_ref[1], ub[pl.ds(128 * i, 128), :], preferred_element_type=F32)

    GI = 4

    def a_conv(g):
        prev = None
        for i0 in range(0, NBLK, GI):
            ys = []
            for ab in range(2):
                r_re, r_im = pl.ds(32 * g + 16 * ab, 8), pl.ds(32 * g + 16 * ab + 8, 8)
                acc = [None] * GI
                uwin = {}
                for m in range(i0 + GI):
                    hr, hi = hh[m, r_re, :], hh[m, r_im, :]
                    for t in range(GI):
                        n = i0 + t - m
                        if n < 0:
                            continue
                        if n not in uwin:
                            uwin[n] = (uh[n, r_re, :], uh[n, r_im, :])
                        ur, ui = uwin[n]
                        pr = hr * ur - hi * ui
                        pi = hr * ui + hi * ur
                        acc[t] = (pr, pi) if acc[t] is None else (acc[t][0] + pr, acc[t][1] + pi)
                ys.append(acc)
            for t in range(GI):
                (ar, ai), (br, bi) = ys[0][t], ys[1][t]
                cur = (ar + br, ai + bi, ar - br, ai - bi)
                if prev is None:
                    res = cur
                elif g < 4:
                    res = (cur[0] - prev[1], cur[1] + prev[0], cur[2] - prev[3], cur[3] + prev[2])
                else:
                    res = (cur[0] + prev[1], cur[1] - prev[0], cur[2] + prev[3], cur[3] - prev[2])
                prev = cur
                eo[i0 + t, 0, pl.ds(16 * g, 16), :] = jnp.concatenate(res[0:2], axis=0).astype(BF16)
                eo[i0 + t, 1, pl.ds(16 * g, 16), :] = jnp.concatenate(res[2:4], axis=0).astype(BF16)

    outa32 = outa.bitcast(U32)

    def a_inv(i):
        ye = jnp.dot(inv_ref[0], eo[i, 0], preferred_element_type=F32)
        yo = jnp.dot(inv_ref[1], eo[i, 1], preferred_element_type=F32)
        rows = pl.ds(64 * i, 64)
        wq = q32[rows, :]
        ae = (ye + uf[0, rows, :]) * _lo(wq)
        ao = (yo + uf[1, rows, :]) * _hi(wq)
        outa32[slot, rows, :] = pltpu.pack_elementwise([ae, ao], packed_dtype=BF16)

    NCH = 256

    def b_qkv(sb, p, c2):
        r0 = sb * SUB
        acc = None
        for kt in range(8):
            part = jax.lax.dot_general(
                x_ref[pl.ds(r0, SUB), pl.ds(128 * kt, 128)],
                wt[kt, pl.ds(p * D + c2 * NCH, NCH), :], NT, preferred_element_type=F32)
            acc = part if acc is None else acc + part
        dst, off = ((qs, 0), (ks, HALO), (vs, HALO))[p]
        for j in range(NCH // 128):
            dst[c2 * (NCH // 128) + j, pl.ds(off + r0, SUB), :] = acc[:, 128 * j:128 * (j + 1)]

    cexp = float(DH ** -0.5 * np.log2(np.e))

    def b_attn(rt2):
        outs = []
        for rt in (2 * rt2, 2 * rt2 + 1):
            r0 = 8 * rt
            qv = [qs[c, pl.ds(r0, 8), :] for c in range(8)]
            lg = []
            for w in range(WIN):
                acc = None
                for c in range(8):
                    pr = qv[c] * ks[c, pl.ds(HALO + r0 - DIL * w, 8), :]
                    acc = pr if acc is None else acc + pr
                acc = acc + pltpu.roll(acc, 64, 1)
                acc = acc + pltpu.roll(acc, 32, 1)
                acc = acc * cexp
                if r0 < DIL * w:
                    acc = jnp.where(row8 + (step * RB + r0) >= DIL * w, acc, -1e9)
                lg.append(acc)
            mx = functools.reduce(jnp.maximum, lg)
            ex = [jnp.exp2(l - mx) for l in lg]
            den = functools.reduce(lambda a, b: a + b, ex)
            rinv = pl.reciprocal(den, approx=True)
            rinv = rinv * (2.0 - den * rinv)
            o = []
            for c in range(8):
                acc = None
                for w in range(WIN):
                    pr = ex[w] * vs[c, pl.ds(HALO + r0 - DIL * w, 8), :]
                    acc = pr if acc is None else acc + pr
                o.append(acc * rinv)
            outs.append(o)
        for c in range(8):
            ob[c, pl.ds(16 * rt2, 16), :] = jnp.concatenate(
                [outs[0][c], outs[1][c]], axis=0).astype(BF16)

    def b_out(sb, c):
        r0 = sb * SUB
        acc = None
        for kt in range(8):
            part = jnp.dot(ob[kt, pl.ds(r0, SUB), :], wop[c, pl.ds(128 * kt, 128), :],
                           preferred_element_type=F32)
            acc = part if acc is None else acc + part
        outb[slot, pl.ds(r0, SUB), pl.ds(128 * c, 128)] = acc.astype(BF16)

    for i in range(NBLK):
        a_fwd_h(i)
        a_prep(i)
    for i in range(NBLK):
        a_fwd_u(i)
    chunks = [(p, c2) for p in range(3) for c2 in range(D // NCH)]
    for n, (p, c2) in enumerate(chunks):
        b_qkv(0, p, c2)
        if n < 6:
            a_conv(n)
    for n, (p, c2) in enumerate(chunks):
        b_qkv(1, p, c2)
        if n < 8:
            b_attn(n)
        elif n < 10:
            a_conv(n - 2)
    for c in range(8):
        b_out(0, c)
        b_attn(8 + c)
    for i in range(NBLK):
        a_inv(i)
    for c in range(8):
        b_out(1, c)
    ks[:, pl.ds(0, HALO), :] = ks[:, pl.ds(RB, HALO), :]
    vs[:, pl.ds(0, HALO), :] = vs[:, pl.ds(RB, HALO), :]

    outa_copy(slot, step).start()
    outb_copy(slot, step).start()

    @pl.when(step == NSTEP - 1)
    def _():
        outa_copy(1 - slot, step - 1).wait()
        outb_copy(1 - slot, step - 1).wait()
        outa_copy(slot, step).wait()
        outb_copy(slot, step).wait()


@jax.jit
def pallas_concat_heads__ssm_conv_h3__sliding_local_dilated__prompt_kernel(
    A_q: jax.Array,
    A_k: jax.Array,
    A_v: jax.Array,
    A_shift_k: jax.Array,
    A_ssm_k: jax.Array,
    A_ssm_D: jax.Array,
    B_x: jax.Array,
    B_wqkv: jax.Array,
    B_wo: jax.Array,
):
    fw, inv, perm = _constants()
    par = jnp.concatenate(
        [A_shift_k.T, A_ssm_D[None, :], jnp.zeros((3, D), A_ssm_D.dtype)], axis=0)
    col = pl.BlockSpec((S, 128), lambda s: (0, s))
    full = lambda a: pl.BlockSpec(a.shape, lambda s: (0,) * a.ndim)
    out = pl.pallas_call(
        _kernel,
        grid=(NSTEP,),
        in_specs=[
            col, col, col,
            pl.BlockSpec((8, 128), lambda s: (0, s)),
            pl.BlockSpec((128, S), lambda s: (s, 0)),
            pl.BlockSpec((RB, D), lambda s: (s, 0)),
            full(fw), full(inv), full(perm),
            pl.BlockSpec(memory_space=pl.ANY),
            pl.BlockSpec(memory_space=pl.ANY),
        ],
        out_specs=pl.BlockSpec(memory_space=pl.ANY),
        out_shape=jax.ShapeDtypeStruct((S, 2 * D), BF16),
        scratch_shapes=[
            pltpu.VMEM((3, D, D), BF16),
            pltpu.VMEM((8, D, 128), BF16),
            pltpu.VMEM((8, 3 * D, 128), BF16),
            pltpu.VMEM((8, D, 128), BF16),
            pltpu.VMEM((8, RB, 128), F32),
            pltpu.VMEM((8, HALO + RB, 128), F32),
            pltpu.VMEM((8, HALO + RB, 128), F32),
            pltpu.VMEM((8, RB, 128), BF16),
            pltpu.VMEM((S, 128), BF16),
            pltpu.VMEM((2, S // 2, 128), F32),
            pltpu.VMEM((NBLK, 256, 128), F32),
            pltpu.VMEM((NBLK, 256, 128), F32),
            pltpu.VMEM((NBLK, 2, 128, 128), BF16),
            pltpu.VMEM((2, S, 128), BF16),
            pltpu.VMEM((2, RB, D), BF16),
            pltpu.SemaphoreType.DMA((11,)),
            pltpu.SemaphoreType.DMA((2, 2)),
        ],
        compiler_params=pltpu.CompilerParams(
            dimension_semantics=("arbitrary",),
            vmem_limit_bytes=100 * 2 ** 20),
    )(A_q[0], A_k[0], A_v[0], par, A_ssm_k, B_x[0], fw, inv, perm, B_wqkv, B_wo)
    return out[None]
```

```python
import functools

import numpy as np
import jax
import jax.numpy as jnp
import jax.experimental.pallas as pl
import jax.experimental.pallas.tpu as pltpu

S = 2048
D = 1024
NH = 32
DH = 32
WIN = 8
DIL = 2
NSTEP = 8
RB = S // NSTEP
SUB = 128
HALO = 16
NBLK = 16
F32 = jnp.float32
BF16 = jnp.bfloat16
U32 = jnp.uint32
NT = (((1,), (1,)), ((), ()))
RATE, QOFF, POFF, ASTEP, REL, XLAT = 2.5, 256, 256, 128, 512, 384


def _constants():
    forder = np.concatenate([np.arange(0, 64, 2), np.arange(1, 64, 2)])
    theta = np.pi * (2 * forder + 1) / 256.0
    j = np.arange(128)
    ang = theta[:, None] * j[None, :]
    sgn = np.where(j % 2 == 0, 1.0, -1.0)[None, :]
    a_re, a_im = np.cos(ang), -np.sin(ang)
    b_re, b_im = a_re * sgn, a_im * sgn
    fwd = np.zeros((256, 128))
    for g in range(8):
        sl = slice(8 * g, 8 * g + 8)
        fwd[32 * g + 0:32 * g + 8] = a_re[sl]
        fwd[32 * g + 8:32 * g + 16] = a_im[sl]
        fwd[32 * g + 16:32 * g + 24] = b_re[sl]
        fwd[32 * g + 24:32 * g + 32] = b_im[sl]
    inv = np.zeros((2, 64, 128))
    s = np.arange(64)
    for p in range(2):
        a = (2 * s + p)[:, None] * theta[None, :]
        inv[p, :, 0::2] = np.cos(a) / 128.0
        inv[p, :, 1::2] = -np.sin(a) / 128.0
    perm = np.zeros((2, 128, 128))
    for jj in range(16):
        for r in range(8):
            hh = r % 4
            perm[0, 8 * jj + r, hh * 32 + 2 * jj + (r // 4)] = 1.0
            perm[1, 8 * jj + r, hh * 32 + 2 * jj + 1 - (r // 4)] = 1.0
    return (jnp.asarray(fwd, BF16), jnp.asarray(inv, BF16), jnp.asarray(perm, BF16))


def _lo(w):
    return pltpu.bitcast(w << 16, F32)


def _hi(w):
    return pltpu.bitcast(w & jnp.uint32(0xFFFF0000), F32)


def _ldb(ref32, *idx):
    return pltpu.bitcast(ref32[idx], BF16)


def _pk(a, b):
    return pltpu.pack_elementwise([a, b], packed_dtype=BF16)


def _kernel(q_ref, k_ref, v_ref, par_ref, h_ref, x_ref, fw_ref, inv_ref, perm_ref,
            wqkv_hbm, wo_hbm, out_hbm,
            wraw, woraw, wt, wop, qs0, qs1, ks0, ks1, vs0, vs1, ob0, ob1, xb, ub, uf, uh, hh, eo, outa, outb,
            wsem, osem):
    step = pl.program_id(0)
    slot = step % 2

    def outa_copy(sl, st):
        return pltpu.make_async_copy(
            outa.at[sl], out_hbm.at[:, pl.ds(pl.multiple_of(st * 128, 128), 128)], osem.at[0, sl])

    def outb_copy(sl, st, c):
        return pltpu.make_async_copy(
            outb.at[sl, c],
            out_hbm.at[pl.ds(pl.multiple_of(st * RB, RB), RB), pl.ds(D + 128 * c, 128)],
            osem.at[1 + c, sl])

    def out_copies(sl, st):
        return [outa_copy(sl, st)] + [outb_copy(sl, st, c) for c in range(8)]

    @pl.when(step == 0)
    def _prologue():
        cps = [pltpu.make_async_copy(wqkv_hbm.at[:, pl.ds(p * D, D)], wraw.at[p], wsem.at[p])
               for p in range(3)]
        cpo = [pltpu.make_async_copy(wo_hbm.at[:, pl.ds(128 * c, 128)], woraw.at[c],
                                     wsem.at[3 + c]) for c in range(8)]
        for cp in cps + cpo:
            cp.start()
        ks0[0, :, pl.ds(0, HALO), :] = jnp.zeros((8, HALO, 128), F32)
        vs0[0, :, pl.ds(0, HALO), :] = jnp.zeros((8, HALO, 128), F32)
        low = jax.lax.broadcasted_iota(jnp.int32, (16, 8, 128), 1) < 4
        for p in range(3):
            cps[p].wait()

            def body(kt, carry, p=p):
                k0 = pl.multiple_of(kt * 128, 128)
                for h4 in range(2):
                    ev, od = [], []
                    for h3 in range(2):
                        t = h4 * 4 + h3 * 2
                        s0 = jax.lax.dot_general(
                            perm_ref[0], wraw[p, pl.ds(k0, 128), pl.ds(128 * t, 128)], NT,
                            preferred_element_type=F32).reshape(16, 8, 128)
                        s1 = jax.lax.dot_general(
                            perm_ref[1], wraw[p, pl.ds(k0, 128), pl.ds(128 * (t + 1), 128)], NT,
                            preferred_element_type=F32).reshape(16, 8, 128)
                        ev.append(jnp.where(low, s0, s1))
                        od.append(pltpu.roll(jnp.where(low, s1, s0), 4, 1))
                    for jj in range(16):
                        for par, src in ((0, ev), (1, od)):
                            row = p * D + (2 * jj + par) * 32 + h4 * 16
                            blk = jnp.concatenate([src[0][jj], src[1][jj]], axis=0)
                            wt[kt, pl.ds(row, 16), :] = blk.astype(BF16)
                return carry

            jax.lax.fori_loop(0, 8, body, 0)
        for cp in cpo:
            cp.wait()
        wo32 = woraw.bitcast(U32)
        wop32 = wop.bitcast(U32)

        def body2(c, carry):
            for dd in range(16):
                for h4 in range(2):
                    a = wo32[c, pl.ds(h4 * 256 + dd, 8, stride=32), :]
                    b = wo32[c, pl.ds(h4 * 256 + 16 + dd, 8, stride=32), :]
                    wop32[c, pl.ds((2 * dd) * 16 + h4 * 8, 8), :] = (
                        (a & jnp.uint32(0xFFFF)) | (b << 16))
                    wop32[c, pl.ds((2 * dd + 1) * 16 + h4 * 8, 8), :] = (
                        (a >> 16) | (b & jnp.uint32(0xFFFF0000)))
            return carry

        jax.lax.fori_loop(0, 8, body2, 0)

    @pl.when(step >= 2)
    def _():
        for cp in out_copies(slot, step - 2):
            cp.wait()

    al = slice(None)
    zero = step // NSTEP
    xz, ufz, eoz = (r.at[zero] for r in (xb, uf, eo))
    hz, uz = hh, uh
    obz = [r.at[zero] for r in (ob0, ob1)]
    hh, uh, xb, ub, uf, eo = (r.at[0] for r in (hh, uh, xb, ub, uf, eo))
    ob = [r.at[0] for r in (ob0, ob1)]
    fw32, inv32 = fw_ref.bitcast(U32), inv_ref.bitcast(U32)
    wt32, wop32 = wt.bitcast(U32), wop.bitcast(U32)
    for kt in range(8):
        xb[kt] = pltpu.bitcast(x_ref[:, pl.ds(128 * kt, 128)], U32)
    k32 = k_ref.bitcast(U32)
    v32 = v_ref.bitcast(U32)
    q32 = q_ref.bitcast(U32)
    par = par_ref[...].astype(F32)
    taps = [jnp.broadcast_to(par[j:j + 1, :], (8, 128)) for j in range(5)]
    row8 = jax.lax.broadcasted_iota(jnp.int32, (8, 128), 0)

    always = perm_ref.bitcast(U32)[0, pl.ds(0, 8), :] != jnp.uint32(0x12345678)

    pend = []
    tnow = [0.0, 0.0]

    clock = []

    def stamp(val, t0):
        for j in range(0, 16, 4):
            clock.append([tnow[0] + t0 + 8 * j, val[8 * j:8 * j + 8], None])

    def release():
        past = [e for e in clock if e[0] <= tnow[1] - REL]
        if not past:
            return zero
        if past[-1][2] is None:
            past[-1][2] = jnp.where(zero == 0, zero, pltpu.bitcast(past[-1][1], jnp.int32)[0, 0])
        return past[-1][2]

    def due(val, ops, extra=0):
        tnow[1] += ops / RATE
        pend.append((tnow[1] + extra, val))
        pend.sort(key=lambda e: e[0])

    def lhs(ref, r0):
        tiles = [[ref[kt, pl.ds(r0 // 2 + 8 * j, 8), :] for j in range(8)] for kt in range(8)]
        n = 0
        while pend and pend[0][0] < tnow[0] + 256:
            t, val = pend.pop(0)
            idx = max(int(t - tnow[0]), 0) // 16
            kt, j = 4 * (idx // 8) + n % 4, idx % 8
            tiles[kt][j] = jnp.where(always, tiles[kt][j], pltpu.bitcast(val, U32))
            n += 1
        return [pltpu.bitcast(jnp.concatenate(t, axis=0), BF16) for t in tiles]

    def a_fwd_h(m):
        r = jax.lax.dot_general(_ldb(fw32, al, al), h_ref[:, pl.ds(128 * m, 128)], NT,
                                preferred_element_type=F32)
        hh[m] = r

    def a_prep(i):
        tp = taps
        for r in range(8 * i, 8 * i + 8):
            w0 = k32[pl.ds(8 * r, 8), :]
            if r == 0:
                w1 = jnp.where(row8 < 1, jnp.uint32(0), pltpu.roll(w0, 1, 0))
                w2 = jnp.where(row8 < 2, jnp.uint32(0), pltpu.roll(w0, 2, 0))
            else:
                w1 = k32[pl.ds(8 * r - 1, 8), :]
                w2 = k32[pl.ds(8 * r - 2, 8), :]
            e0, o0, e1, o1, o2 = _lo(w0), _hi(w0), _lo(w1), _hi(w1), _hi(w2)
            kse = tp[0] * e0 + tp[1] * o1 + tp[2] * e1 + tp[3] * o2
            kso = tp[0] * o0 + tp[1] * e0 + tp[2] * o1 + tp[3] * e1
            wv = v32[pl.ds(8 * r, 8), :]
            ue = kse * _lo(wv)
            uo = kso * _hi(wv)
            pk = _pk(ue, uo)
            ub[pl.ds(8 * r, 8), :] = pk
            uf[0, pl.ds(8 * r, 8), :] = ue * taps[4]
            uf[1, pl.ds(8 * r, 8), :] = uo * taps[4]

    def a_fwd_u(i):
        r = jnp.dot(_ldb(fw32, al, al), _ldb(ub, pl.ds(64 * i, 64), al),
                    preferred_element_type=F32)
        uh[i] = r

    conv_state = {}

    def a_conv(g, i):
        ys = []
        for ab in range(2):
            r_re, r_im = pl.ds(32 * g + 16 * ab, 8), pl.ds(32 * g + 16 * ab + 8, 8)
            z = release()
            for m in range(i + 1):
                hr, hi = hz[z, m, r_re, :], hz[z, m, r_im, :]
                ur, ui = uz[z, i - m, r_re, :], uz[z, i - m, r_im, :]
                yr = hr * ur if m == 0 else yr + hr * ur
                yi = hr * ui if m == 0 else yi + hr * ui
                yr, yi = yr - hi * ui, yi + hi * ur
            ys.append((yr, yi))
            if ab == 0:
                due(yr, 8 * i + 8)
                due(yi, 0)
        (ar, ai), (br, bi) = ys
        cur = (ar + br, ai + bi, ar - br, ai - bi)
        prev = conv_state.get("prev")
        if i == 0:
            res = cur
        elif g < 4:
            res = (cur[0] - prev[1], cur[1] + prev[0], cur[2] - prev[3], cur[3] + prev[2])
        else:
            res = (cur[0] + prev[1], cur[1] - prev[0], cur[2] + prev[3], cur[3] - prev[2])
        conv_state["prev"] = cur
        pe, po = _pk(res[0], res[1]), _pk(res[2], res[3])
        eo[i, 0, pl.ds(8 * g, 8), :] = pe
        eo[i, 1, pl.ds(8 * g, 8), :] = po
        due(pe, 8 * i + 18)
        due(po, 0)

    outa32 = outa.bitcast(U32)

    def a_inv(i):
        ye = jnp.dot(_ldb(inv32, 0), _ldb(eoz, i, 0), preferred_element_type=F32)
        yo = jnp.dot(_ldb(inv32, 1), _ldb(eoz, i, 1), preferred_element_type=F32)
        rows = pl.ds(64 * i, 64)
        wq = q32[rows, :]
        ae = (ye + ufz[0, rows, :]) * _lo(wq)
        ao = (yo + ufz[1, rows, :]) * _hi(wq)
        outa32[slot, rows, :] = _pk(ae, ao)

    NCH = 128
    qs, ks, vs = (qs0, qs1), (ks0, ks1), (vs0, vs1)

    def b_qkv(sb, p, c2):
        r0 = sb * SUB
        acc = None
        xs = lhs(xz, r0)
        for kt in range(8):
            part = jax.lax.dot_general(
                xs[kt],
                _ldb(wt32, kt, pl.ds((p * D + c2 * NCH) // 2, NCH // 2), al), NT, preferred_element_type=F32)
            acc = part if acc is None else acc + part
            if kt % 4 == 3:
                stamp(acc, 32 * (kt - 3))
        if p == 0:
            qs[sb][0, c2] = acc
        else:
            dst = (ks, vs)[p - 1]
            dst[sb][0, c2, pl.ds(HALO, SUB), :] = acc
            dst[1 - sb][0, c2, pl.ds(0, HALO), :] = acc[SUB - HALO:]

    cexp = float(DH ** -0.5 * np.log2(np.e))

    logits = {}
    outs = {}

    def b_rows(rt):
        return 32 * (rt // 4) + (0, 2, 1, 3)[rt % 4]

    def b_qk(rt):
        sb, r0 = rt // 16, b_rows(rt % 16)
        lg = [None] * WIN
        z = release()
        for c in range(8):
            qv = qs[sb][z, c, pl.ds(r0, 8, stride=4), :] * cexp
            for w in range(WIN):
                pr = qv * ks[sb][z, c, pl.ds(HALO - DIL * w + r0, 8, stride=4), :]
                lg[w] = pr if c == 0 else lg[w] + pr
        for w in range(WIN):
            acc = lg[w]
            acc = acc + pltpu.roll(acc, 64, 1)
            acc = acc + pltpu.roll(acc, 32, 1)
            if sb == 0 and r0 < DIL * w:
                acc = jnp.where(4 * row8 + (step * RB + r0) >= DIL * w, acc, -1e9)
            lg[w] = acc
            due(acc, 20, XLAT)
        logits[rt] = lg

    def b_pv(rt):
        sb, r0 = rt // 16, b_rows(rt % 16)
        z = release()
        lg = logits.pop(rt)
        mx = functools.reduce(jnp.maximum, lg)
        ex = [jnp.exp2(l - mx) for l in lg]
        den = functools.reduce(lambda a, b: a + b, ex)
        rinv = pl.reciprocal(den, approx=True)
        rinv = rinv * (2.0 - den * rinv)
        o = [None] * 8
        for w in range(WIN):
            for c in range(8):
                pr = ex[w] * vs[sb][z, c, pl.ds(HALO - DIL * w + r0, 8, stride=4), :]
                o[c] = pr if w == 0 else o[c] + pr
        o = [x * rinv for x in o]
        outs[rt] = o
        if rt % 2 == 1:
            o0, o1 = outs.pop(rt - 1), outs.pop(rt)
            o = [_pk(o0[c], o1[c]) for c in range(8)]
            for c in range(8):
                ob[rt // 16][c, pl.ds(8 * (rt % 16 // 2), 8), :] = o[c]
        for x in o:
            due(x, 21)

    outb32 = outb.bitcast(U32)

    def b_out(sb, c):
        r0 = sb * SUB
        acc = None
        xs = lhs(obz[sb], 0)
        for kt in range(8):
            part = jnp.dot(xs[kt],
                           _ldb(wop32, c, pl.ds(64 * kt, 64), al),
                           preferred_element_type=F32)
            acc = part if acc is None else acc + part
            if kt % 4 == 3:
                stamp(acc, 32 * (kt - 3))
        for j in range(SUB // 32):
            outb32[slot, c, pl.ds(r0 // 2 + 16 * j, 16), :] = _pk(
                acc[32 * j:32 * j + 16], acc[32 * j + 16:32 * j + 32])

    P = functools.partial
    qkv = lambda sb, p, cs=range(8): [(P(b_qkv, sb, p, c), 256) for c in cs]
    mxu = ([(P(a_fwd_h, i), 64) for i in range(NBLK)] + qkv(0, 0, range(2))
           + [(P(a_fwd_u, i), 64) for i in range(NBLK)] + qkv(0, 0, range(2, 8))
           + qkv(0, 1) + qkv(0, 2) + qkv(1, 0) + qkv(1, 1) + qkv(1, 2)
           + [(P(a_inv, i), 32) for i in range(NBLK)]
           + [(P(b_out, 0, c), 256) for c in range(8)]
           + [(P(b_out, 1, c), 256) for c in range(8)])
    vpu = [(512 + 64 * i, P(a_prep, i)) for i in range(NBLK)]
    conv = [(16 * i + 26, P(a_conv, g, i)) for g in range(8) for i in range(NBLK)]
    att = []
    for sb, t0 in ((0, 6144), (1, 12288)):
        att += [(t0 + QOFF + ASTEP * j, 160, P(b_qk, 16 * sb + j)) for j in range(16)]
        att += [(t0 + 2048 + POFF + ASTEP * j, 168, P(b_pv, 16 * sb + j)) for j in range(16)]
    t = 2560.0 + POFF
    while conv or att:
        if att and att[0][0] <= t:
            _, ops, fn = att.pop(0)
        elif conv:
            ops, fn = conv.pop(0)
            assert t < 14080
        else:
            t = att[0][0]
            continue
        vpu.append((t, fn))
        t += ops / RATE
    assert t < 16896
    for fn, cyc in mxu:
        while vpu and vpu[0][0] < tnow[0] + cyc:
            tnow[1], unit = vpu.pop(0)
            unit()
        fn()
        tnow[0] += cyc
    assert not vpu

    for cp in out_copies(slot, step):
        cp.start()

    @pl.when(step == NSTEP - 1)
    def _():
        for cp in out_copies(1 - slot, step - 1) + out_copies(slot, step):
            cp.wait()


@jax.jit
def pallas_concat_heads__ssm_conv_h3__sliding_local_dilated__prompt_kernel(
    A_q: jax.Array,
    A_k: jax.Array,
    A_v: jax.Array,
    A_shift_k: jax.Array,
    A_ssm_k: jax.Array,
    A_ssm_D: jax.Array,
    B_x: jax.Array,
    B_wqkv: jax.Array,
    B_wo: jax.Array,
):
    fw, inv, perm = _constants()
    par = jnp.concatenate(
        [A_shift_k.T, A_ssm_D[None, :], jnp.zeros((3, D), A_ssm_D.dtype)], axis=0)
    col = pl.BlockSpec((S, 128), lambda s: (0, s))
    full = lambda a: pl.BlockSpec(a.shape, lambda s: (0,) * a.ndim)
    out = pl.pallas_call(
        _kernel,
        grid=(NSTEP,),
        in_specs=[
            col, col, col,
            pl.BlockSpec((8, 128), lambda s: (0, s)),
            pl.BlockSpec((128, S), lambda s: (s, 0)),
            pl.BlockSpec((RB, D), lambda s: (s, 0)),
            full(fw), full(inv), full(perm),
            pl.BlockSpec(memory_space=pl.ANY),
            pl.BlockSpec(memory_space=pl.ANY),
        ],
        out_specs=pl.BlockSpec(memory_space=pl.ANY),
        out_shape=jax.ShapeDtypeStruct((S, 2 * D), BF16),
        scratch_shapes=[
            pltpu.VMEM((3, D, D), BF16),
            pltpu.VMEM((8, D, 128), BF16),
            pltpu.VMEM((8, 3 * D, 128), BF16),
            pltpu.VMEM((8, D, 128), BF16),
            pltpu.VMEM((1, 8, SUB, 128), F32),
            pltpu.VMEM((1, 8, SUB, 128), F32),
            pltpu.VMEM((1, 8, HALO + SUB, 128), F32),
            pltpu.VMEM((1, 8, HALO + SUB, 128), F32),
            pltpu.VMEM((1, 8, HALO + SUB, 128), F32),
            pltpu.VMEM((1, 8, HALO + SUB, 128), F32),
            pltpu.VMEM((1, 8, SUB // 2, 128), U32),
            pltpu.VMEM((1, 8, SUB // 2, 128), U32),
            pltpu.VMEM((1, 8, RB // 2, 128), U32),
            pltpu.VMEM((1, S // 2, 128), U32),
            pltpu.VMEM((1, 2, S // 2, 128), F32),
            pltpu.VMEM((1, NBLK, 256, 128), F32),
            pltpu.VMEM((1, NBLK, 256, 128), F32),
            pltpu.VMEM((1, NBLK, 2, 64, 128), U32),
            pltpu.VMEM((2, S, 128), BF16),
            pltpu.VMEM((2, 8, RB, 128), BF16),
            pltpu.SemaphoreType.DMA((11,)),
            pltpu.SemaphoreType.DMA((9, 2)),
        ],
        compiler_params=pltpu.CompilerParams(
            dimension_semantics=("arbitrary",),
            vmem_limit_bytes=100 * 2 ** 20,
            disable_bounds_checks=True),
    )(A_q[0], A_k[0], A_v[0], par, A_ssm_k, B_x[0], fw, inv, perm, B_wqkv, B_wo)
    return out[None]
```

```python
import functools

import numpy as np
import jax
import jax.numpy as jnp
import jax.experimental.pallas as pl
import jax.experimental.pallas.tpu as pltpu

S = 2048
D = 1024
NH = 32
DH = 32
WIN = 8
DIL = 2
NSTEP = 8
RB = S // NSTEP
SUB = 128
HALO = 16
NBLK = 16
F32 = jnp.float32
BF16 = jnp.bfloat16
U32 = jnp.uint32
NT = (((1,), (1,)), ((), ()))
RATE, CRATE, QOFF, POFF, ASTEP, XLAT = 2.0, 2.5, 256, 384, 120, 192


def _constants():
    forder = np.concatenate([np.arange(0, 64, 2), np.arange(1, 64, 2)])
    theta = np.pi * (2 * forder + 1) / 256.0
    j = np.arange(128)
    ang = theta[:, None] * j[None, :]
    sgn = np.where(j % 2 == 0, 1.0, -1.0)[None, :]
    a_re, a_im = np.cos(ang), -np.sin(ang)
    b_re, b_im = a_re * sgn, a_im * sgn
    fwd = np.zeros((256, 128))
    for g in range(8):
        sl = slice(8 * g, 8 * g + 8)
        fwd[32 * g + 0:32 * g + 8] = a_re[sl]
        fwd[32 * g + 8:32 * g + 16] = a_im[sl]
        fwd[32 * g + 16:32 * g + 24] = b_re[sl]
        fwd[32 * g + 24:32 * g + 32] = b_im[sl]
    inv = np.zeros((2, 64, 128))
    s = np.arange(64)
    for p in range(2):
        a = (2 * s + p)[:, None] * theta[None, :]
        inv[p, :, 0::2] = np.cos(a) / 128.0
        inv[p, :, 1::2] = -np.sin(a) / 128.0
    perm = np.zeros((2, 128, 128))
    for jj in range(16):
        for r in range(8):
            hh = r % 4
            perm[0, 8 * jj + r, hh * 32 + 2 * jj + (r // 4)] = 1.0
            perm[1, 8 * jj + r, hh * 32 + 2 * jj + 1 - (r // 4)] = 1.0
    return (jnp.asarray(fwd, BF16), jnp.asarray(inv, BF16), jnp.asarray(perm, BF16))


def _lo(w):
    return pltpu.bitcast(w << 16, F32)


def _hi(w):
    return pltpu.bitcast(w & jnp.uint32(0xFFFF0000), F32)


def _ldb(ref32, *idx):
    return pltpu.bitcast(ref32[idx], BF16)


def _pk(a, b):
    return pltpu.pack_elementwise([a, b], packed_dtype=BF16)


def _kernel(sk_ref, d_ref, fw_ref, inv_ref, perm_ref,
            q_hbm, k_hbm, v_hbm, h_hbm, x_hbm, wqkv_hbm, wo_hbm, out_hbm,
            qin, kin, vin, hin, xin, wraw, woraw, *rest):
    outa, outb, wsem, isem, osem = rest[-5:]
    step = pl.program_id(0)
    slot = step % 2

    def in_copies(st, sl, sems):
        c0 = pl.multiple_of(st * 128, 128)
        pairs = [(h_hbm.at[pl.ds(c0, 128), :], hin), (k_hbm.at[:, pl.ds(c0, 128)], kin),
                 (v_hbm.at[:, pl.ds(c0, 128)], vin),
                 (x_hbm.at[pl.ds(pl.multiple_of(st * RB, RB), RB), :], xin),
                 (q_hbm.at[:, pl.ds(c0, 128)], qin)]
        return [pltpu.make_async_copy(src, dst.at[sl], sem) for (src, dst), sem in zip(pairs, sems)]

    def out_copies(st, sl):
        return [
            pltpu.make_async_copy(
                outa.at[sl], out_hbm.at[:, pl.ds(pl.multiple_of(st * 128, 128), 128)], osem.at[sl]),
            pltpu.make_async_copy(
                outb.at[sl], out_hbm.at[pl.ds(pl.multiple_of(st * RB, RB), RB), pl.ds(D, D)],
                osem.at[sl])]

    nxt = in_copies(jnp.minimum(step + 1, NSTEP - 1), 1 - slot, [isem.at[1 - slot]] * 5)
    bufs = [r.at[slot] for r in (qin, kin, vin, hin, xin, outa, outb)]
    consts = (sk_ref, d_ref, fw_ref, inv_ref, perm_ref)

    @pl.when(step == 0)
    def _():
        dma = dict(zip("hkvxq", in_copies(0, 0, [wsem.at[j] for j in range(5)])))
        for j in range(4):
            rows = pl.ds(256 * j, 256)
            dma[j] = pltpu.make_async_copy(
                wqkv_hbm.at[rows, pl.ds(0, D)], wraw.at[0, rows, :], wsem.at[5 + j])
        for pp in (1, 2):
            dma["w%d" % pp] = pltpu.make_async_copy(
                wqkv_hbm.at[:, pl.ds(pp * D, D)], wraw.at[pp], wsem.at[8 + pp])
        for c in range(8):
            dma["o%d" % c] = pltpu.make_async_copy(
                wo_hbm.at[:, pl.ds(128 * c, 128)], woraw.at[c], wsem.at[11])
        for j, cp in enumerate(nxt):
            dma["n%d" % j] = cp
        _body(step, consts, bufs, (wraw, woraw), rest[:-5], dma)

    @pl.when(step >= 2)
    def _():
        for cp in out_copies(step - 2, slot):
            cp.wait()

    @pl.when(step > 0)
    def _():
        for cp in in_copies(step, slot, [isem.at[slot]] * 5):
            cp.wait()
        for cp in nxt:
            cp.start()
        _body(step, consts, bufs, None, rest[:-5], None)

    for cp in out_copies(step, slot):
        cp.start()

    @pl.when(step == NSTEP - 1)
    def _():
        for cp in nxt + out_copies(step - 1, 1 - slot) + out_copies(step, slot):
            cp.wait()


def _body(step, consts, bufs, wsrc, scratch, dma):
    sk_ref, d_ref, fw_ref, inv_ref, perm_ref = consts
    q_ref, k_ref, v_ref, h_ref, x_ref, outa, outb = bufs
    wt0, wt1, wt2, wop, qs0, qs1, ks0, ks1, vs0, vs1, ob0, ob1, xb, ub, uf, hu, eo = scratch
    first = dma is not None
    al = slice(None)
    zero = step // NSTEP
    xz, ufz, eoz = (r.at[zero] for r in (xb, uf, eo))
    obz = [r.at[zero] for r in (ob0, ob1)]
    xb, ub, uf, eo = (r.at[0] for r in (xb, ub, uf, eo))
    ob = [r.at[0] for r in (ob0, ob1)]
    fw32, inv32 = fw_ref.bitcast(U32), inv_ref.bitcast(U32)
    wt32 = [r.bitcast(U32).at[zero] for r in (wt0, wt1, wt2)]
    wop32 = wop.at[zero]
    perm32 = perm_ref.bitcast(U32)
    k32 = k_ref.bitcast(U32)
    v32 = v_ref.bitcast(U32)
    q32 = q_ref.bitcast(U32)
    row8 = jax.lax.broadcasted_iota(jnp.int32, (8, 128), 0)
    sk = sk_ref[:, pl.ds(pl.multiple_of(step * 128, 128), 128)].astype(F32)
    taps = [jnp.broadcast_to(sk[j:j + 1, :], (8, 128)) for j in range(4)]
    dall = d_ref[...].astype(F32).reshape(8, 128)
    taps.append(jnp.broadcast_to(
        jnp.sum(jnp.where(row8 == step, dall, 0.0), axis=0, keepdims=True), (8, 128)))

    always = perm32[0, pl.ds(0, 8), :] != jnp.uint32(0x12345678)

    pend = []
    tnow = [0.0, 0.0, 1.0]

    cnt = [1]

    def fresh():
        cnt[0] += 1
        return zero * cnt[0]

    def due(val, ops, extra=0):
        tnow[1] += ops / tnow[2]
        pend.append((tnow[1] + extra, val))
        pend.sort(key=lambda e: e[0])

    def lhs(ref, r0, mod=8):
        tiles = [[ref[kt % mod, pl.ds(r0 // 2 + 8 * j, 8), :] for j in range(8)] for kt in range(8)]
        n = 0
        while pend and pend[0][0] < tnow[0] + 256:
            t, val = pend.pop(0)
            idx = max(int(t - tnow[0]), 0) // 16
            kt, j = 4 * (idx // 8) + n % 4, idx % 8
            tiles[kt][j] = jnp.where(always, tiles[kt][j], pltpu.bitcast(val, U32))
            n += 1
        return [pltpu.bitcast(jnp.concatenate(t, axis=0), BF16) for t in tiles]

    def a_fwd_h(m):
        r = jax.lax.dot_general(_ldb(fw32, al, al), h_ref[:, pl.ds(128 * m, 128)], NT,
                                preferred_element_type=F32)
        hu[0, m] = r

    def a_prep(i):
        tp = taps
        for r in range(8 * i, 8 * i + 8):
            w0 = k32[pl.ds(8 * r, 8), :]
            if r == 0:
                w1 = jnp.where(row8 < 1, jnp.uint32(0), pltpu.roll(w0, 1, 0))
                w2 = jnp.where(row8 < 2, jnp.uint32(0), pltpu.roll(w0, 2, 0))
            else:
                w1 = k32[pl.ds(8 * r - 1, 8), :]
                w2 = k32[pl.ds(8 * r - 2, 8), :]
            e0, o0, e1, o1, o2 = _lo(w0), _hi(w0), _lo(w1), _hi(w1), _hi(w2)
            kse = tp[0] * e0 + tp[1] * o1 + tp[2] * e1 + tp[3] * o2
            kso = tp[0] * o0 + tp[1] * e0 + tp[2] * o1 + tp[3] * e1
            wv = v32[pl.ds(8 * r, 8), :]
            ue = kse * _lo(wv)
            uo = kso * _hi(wv)
            pk = _pk(ue, uo)
            ub[pl.ds(8 * r, 8), :] = pk
            uf[0, pl.ds(8 * r, 8), :] = ue * taps[4]
            uf[1, pl.ds(8 * r, 8), :] = uo * taps[4]

    def a_fwd_u(i):
        r = jnp.dot(_ldb(fw32, al, al), _ldb(ub, pl.ds(64 * i, 64), al),
                    preferred_element_type=F32)
        hu[0, NBLK + i] = r

    conv_state = {}

    def a_conv(g, i):
        ys = []
        for ab in range(2):
            z = fresh()
            r_re, r_im = pl.ds(32 * g + 16 * ab, 8), pl.ds(32 * g + 16 * ab + 8, 8)
            for m in range(i + 1):
                hr, hi = hu[z, m, r_re, :], hu[z, m, r_im, :]
                ur, ui = hu[z, NBLK + i - m, r_re, :], hu[z, NBLK + i - m, r_im, :]
                yr = hr * ur if m == 0 else yr + hr * ur
                yi = hr * ui if m == 0 else yi + hr * ui
                yr, yi = yr - hi * ui, yi + hi * ur
            ys.append((yr, yi))
            if ab == 0:
                due(yr, 8 * i + 8)
                due(yi, 0)
        (ar, ai), (br, bi) = ys
        cur = (ar + br, ai + bi, ar - br, ai - bi)
        prev = conv_state.get("prev")
        if i == 0:
            res = cur
        elif g < 4:
            res = (cur[0] - prev[1], cur[1] + prev[0], cur[2] - prev[3], cur[3] + prev[2])
        else:
            res = (cur[0] + prev[1], cur[1] - prev[0], cur[2] + prev[3], cur[3] - prev[2])
        conv_state["prev"] = cur
        pe, po = _pk(res[0], res[1]), _pk(res[2], res[3])
        eo[i, 0, pl.ds(8 * g, 8), :] = pe
        eo[i, 1, pl.ds(8 * g, 8), :] = po
        due(pe, 8 * i + 18)
        due(po, 0)

    outa32 = outa.bitcast(U32)

    def a_inv(i):
        ye = jnp.dot(_ldb(inv32, 0), _ldb(eoz, i, 0), preferred_element_type=F32)
        yo = jnp.dot(_ldb(inv32, 1), _ldb(eoz, i, 1), preferred_element_type=F32)
        rows = pl.ds(64 * i, 64)
        wq = q32[rows, :]
        ae = (ye + ufz[0, rows, :]) * _lo(wq)
        ao = (yo + ufz[1, rows, :]) * _hi(wq)
        outa32[rows, :] = _pk(ae, ao)

    qs, ks, vs = (qs0, qs1), (ks0, ks1), (vs0, vs1)

    def b_qkv(sb, p, c2):
        r0 = sb * SUB
        acc = None
        xs = lhs(xz, r0)
        for kt in range(8):
            part = jax.lax.dot_general(
                xs[kt],
                _ldb(wt32[p], kt, pl.ds(c2 * 64, 64), al), NT,
                preferred_element_type=F32)
            acc = part if acc is None else acc + part
        if p == 0:
            qs[sb][0, c2] = acc
        else:
            dst = (ks, vs)[p - 1]
            dst[sb][0, c2, pl.ds(HALO, SUB), :] = acc
            if sb == 0:
                dst[1][0, c2, pl.ds(0, HALO), :] = acc[SUB - HALO:]

    cexp = float(DH ** -0.5 * np.log2(np.e))

    logits = {}
    outs = {}

    def b_rows(rt):
        return 32 * (rt // 4) + (0, 2, 1, 3)[rt % 4]

    def b_qk(rt):
        sb, r0 = rt // 16, b_rows(rt % 16)
        lg = [None] * WIN
        z = fresh()
        for c in range(8):
            qv = qs[sb][z, c, pl.ds(r0, 8, stride=4), :] * cexp
            for w in range(WIN):
                pr = qv * ks[sb][z, c, pl.ds(HALO - DIL * w + r0, 8, stride=4), :]
                lg[w] = pr if c == 0 else lg[w] + pr
        logits[rt] = [x + pltpu.roll(x, 64, 1) for x in lg]
        for x in logits[rt][3::4]:
            due(x, 72, XLAT)

    def b_q2(rt):
        sb, r0 = rt // 16, b_rows(rt % 16)
        lg = logits[rt]
        for w in range(WIN):
            acc = lg[w] + pltpu.roll(lg[w], 32, 1)
            if sb == 0 and r0 < DIL * w:
                acc = jnp.where(4 * row8 + (step * RB + r0) >= DIL * w, acc, -1e9)
            lg[w] = acc
            due(acc, 2, XLAT)

    def b_pv(rt):
        sb, r0 = rt // 16, b_rows(rt % 16)
        z = fresh()
        lg = logits.pop(rt)
        mx = functools.reduce(jnp.maximum, lg)
        ex = [jnp.exp2(l - mx) for l in lg]
        den = functools.reduce(lambda a, b: a + b, ex)
        rinv = pl.reciprocal(den, approx=True)
        rinv = rinv * (2.0 - den * rinv)
        o = [None] * 8
        for w in range(WIN):
            for c in range(8):
                pr = ex[w] * vs[sb][z, c, pl.ds(HALO - DIL * w + r0, 8, stride=4), :]
                o[c] = pr if w == 0 else o[c] + pr
        o = [x * rinv for x in o]
        outs[rt] = o
        if rt % 2 == 1:
            o0, o1 = outs.pop(rt - 1), outs.pop(rt)
            o = [_pk(o0[c], o1[c]) for c in range(8)]
            for c in range(8):
                ob[rt // 16][c, pl.ds(8 * (rt % 16 // 2), 8), :] = o[c]
        for x in o:
            due(x, 21)

    def b_out(sb, c):
        r0 = sb * SUB
        acc = None
        xs = lhs(obz[sb], 0)
        for kt in range(8):
            part = jnp.dot(xs[kt],
                           _ldb(wop32, c, pl.ds(64 * kt, 64), al),
                           preferred_element_type=F32)
            acc = part if acc is None else acc + part
        for j in range(SUB // 32):
            outb[pl.ds(r0 + 32 * j, 32), pl.ds(128 * c, 128)] = pltpu.bitcast(_pk(
                acc[32 * j:32 * j + 16], acc[32 * j + 16:32 * j + 32]), BF16)

    def b_x():
        for kt in range(8):
            xb[kt] = pltpu.bitcast(x_ref[:, pl.ds(128 * kt, 128)], U32)

    def w_perm(p, kt):
        low = jax.lax.broadcasted_iota(jnp.int32, (16, 8, 128), 1) < 4
        sel = lhs(perm32, 0, 2)
        tr = [jax.lax.dot_general(
            sel[t], wsrc[0][p, pl.ds(128 * kt, 128), pl.ds(128 * t, 128)], NT,
            preferred_element_type=F32).reshape(16, 8, 128) for t in range(8)]
        for h4 in range(2):
            ev = [jnp.where(low, tr[t], tr[t + 1]) for t in (4 * h4, 4 * h4 + 2)]
            od = [pltpu.roll(jnp.where(low, tr[t + 1], tr[t]), 4, 1) for t in (4 * h4, 4 * h4 + 2)]
            for jj in range(16):
                for par, src in ((0, ev), (1, od)):
                    blk = jnp.concatenate([src[0][jj], src[1][jj]], axis=0)
                    (wt0, wt1, wt2)[p][0, kt, pl.ds((2 * jj + par) * 32 + h4 * 16, 16), :] = (
                        blk.astype(BF16))

    def wo_perm(c):
        wo32 = wsrc[1].bitcast(U32)
        for dd in range(16):
            for h4 in range(2):
                a = wo32[c, pl.ds(h4 * 256 + dd, 8, stride=32), :]
                b = wo32[c, pl.ds(h4 * 256 + 16 + dd, 8, stride=32), :]
                wop[0, c, pl.ds((2 * dd) * 16 + h4 * 8, 8), :] = (
                    (a & jnp.uint32(0xFFFF)) | (b << 16))
                wop[0, c, pl.ds((2 * dd + 1) * 16 + h4 * 8, 8), :] = (
                    (a >> 16) | (b & jnp.uint32(0xFFFF0000)))

    def sync(wait, start):
        for key in wait:
            dma[key].wait()
        for key in start:
            dma[key].start()

    P = functools.partial
    qkv = lambda sb, p, cs=range(8): [(P(b_qkv, sb, p, c), 256) for c in cs]
    fwd_h = [(P(a_fwd_h, i), 64) for i in range(NBLK)]
    fwd_u = [(P(a_fwd_u, i), 64) for i in range(NBLK)]
    tail = ([(P(a_inv, i), 32) for i in range(NBLK)]
            + [(P(b_out, sb, c), 256) for sb in range(2) for c in range(8)])

    def conv(t):
        for g in range(8):
            for i in range(NBLK):
                vpu.append((t, CRATE, P(a_conv, g, i)))
                t += (16 * i + 26) / CRATE

    def att(fn, sb, t, dt):
        vpu.extend((t + dt * j, RATE, P(fn, 16 * sb + j)) for j in range(16))

    if first:
        ks0[0, :, pl.ds(0, HALO), :] = jnp.zeros((8, HALO, 128), F32)
        vs0[0, :, pl.ds(0, HALO), :] = jnp.zeros((8, HALO, 128), F32)
        wos = ["o%d" % c for c in range(8)]
        perm = lambda p, kts=range(8): [(P(w_perm, p, kt), 256) for kt in kts]
        sy = lambda wait, start=(): [(P(sync, wait, start), 0)]
        mxu = (sy([], [0, 1, 2, 3, "x"]) + sy([0], "hkv") + perm(0, (0, 1)) + sy([1], ["w1"])
               + perm(0, (2, 3)) + sy([2]) + perm(0, (4, 5)) + sy([3, "x"], ["w2"])
               + [(b_x, 0)] + perm(0, (6, 7)) + qkv(0, 0) + qkv(1, 0, range(4))
               + sy("hkv", ["q"] + wos) + fwd_h + qkv(1, 0, range(4, 8)) + fwd_u
               + sy(["w1"], ["n%d" % j for j in range(5)]) + perm(1) + qkv(0, 1) + qkv(1, 1)
               + sy(["w2"]) + perm(2) + qkv(0, 2) + sy(["q"] + wos) + qkv(1, 2) + tail)
        vpu = [(6144 + 64 * i, 1, P(a_prep, i)) for i in range(NBLK)]
        conv(8192.0 + POFF)
        for sb in range(2):
            att(b_qk, sb, 14336 + QOFF + 2048 * sb, ASTEP)
            att(b_q2, sb, 14336 + QOFF + 2048 * sb + 260, ASTEP)
            att(b_pv, sb, 18432 + POFF + 2048 * sb, ASTEP)
        vpu += [(18432 + 256 * c, 1, P(wo_perm, c)) for c in range(8)]
    else:
        mxu = ([(b_x, 0)] + fwd_h + qkv(0, 2, range(2)) + fwd_u + qkv(0, 2, range(2, 8))
               + qkv(0, 0) + qkv(0, 1) + qkv(1, 0) + qkv(1, 1) + qkv(1, 2) + tail)
        vpu = [(512 + 64 * i, 1, P(a_prep, i)) for i in range(NBLK)]
        conv(2560.0 + POFF)
        att(b_qk, 0, 8192 + QOFF, 224)
        att(b_q2, 0, 8192 + QOFF + 230, 224)
        att(b_pv, 0, 8192 + QOFF + 560, 224)
        att(b_qk, 1, 12288 + QOFF, ASTEP)
        att(b_q2, 1, 12288 + QOFF + 260, ASTEP)
        att(b_pv, 1, 14336 + POFF, ASTEP)
    vpu.sort(key=lambda e: e[0])
    for fn, cyc in mxu:
        while vpu and vpu[0][0] < tnow[0] + cyc:
            tnow[1], tnow[2], unit = vpu.pop(0)
            unit()
        fn()
        tnow[0] += cyc
    assert not vpu
    ks0[0, :, pl.ds(0, HALO), :] = ks1[0, :, pl.ds(SUB, HALO), :]
    vs0[0, :, pl.ds(0, HALO), :] = vs1[0, :, pl.ds(SUB, HALO), :]


@jax.jit
def pallas_concat_heads__ssm_conv_h3__sliding_local_dilated__prompt_kernel(
    A_q: jax.Array,
    A_k: jax.Array,
    A_v: jax.Array,
    A_shift_k: jax.Array,
    A_ssm_k: jax.Array,
    A_ssm_D: jax.Array,
    B_x: jax.Array,
    B_wqkv: jax.Array,
    B_wo: jax.Array,
):
    fw, inv, perm = _constants()
    small = (A_shift_k.T, A_ssm_D, fw, inv, perm)
    full = lambda a: pl.BlockSpec(a.shape, lambda s: (0,) * a.ndim)
    out = pl.pallas_call(
        _kernel,
        grid=(NSTEP,),
        in_specs=[full(a) for a in small] + [pl.BlockSpec(memory_space=pl.ANY)] * 7,
        out_specs=pl.BlockSpec(memory_space=pl.ANY),
        out_shape=jax.ShapeDtypeStruct((S, 2 * D), BF16),
        scratch_shapes=[
            pltpu.VMEM((2, S, 128), BF16),
            pltpu.VMEM((2, S, 128), BF16),
            pltpu.VMEM((2, S, 128), BF16),
            pltpu.VMEM((2, 128, S), BF16),
            pltpu.VMEM((2, RB, D), BF16),
            pltpu.VMEM((3, D, D), BF16),
            pltpu.VMEM((8, D, 128), BF16),
            pltpu.VMEM((1, 8, D, 128), BF16),
            pltpu.VMEM((1, 8, D, 128), BF16),
            pltpu.VMEM((1, 8, D, 128), BF16),
            pltpu.VMEM((1, 8, D // 2, 128), U32),
            pltpu.VMEM((1, 8, SUB, 128), F32),
            pltpu.VMEM((1, 8, SUB, 128), F32),
            pltpu.VMEM((1, 8, HALO + SUB, 128), F32),
            pltpu.VMEM((1, 8, HALO + SUB, 128), F32),
            pltpu.VMEM((1, 8, HALO + SUB, 128), F32),
            pltpu.VMEM((1, 8, HALO + SUB, 128), F32),
            pltpu.VMEM((1, 8, SUB // 2, 128), U32),
            pltpu.VMEM((1, 8, SUB // 2, 128), U32),
            pltpu.VMEM((1, 8, RB // 2, 128), U32),
            pltpu.VMEM((1, S // 2, 128), U32),
            pltpu.VMEM((1, 2, S // 2, 128), F32),
            pltpu.VMEM((1, 2 * NBLK, 256, 128), F32),
            pltpu.VMEM((1, NBLK, 2, 64, 128), U32),
            pltpu.VMEM((2, S, 128), BF16),
            pltpu.VMEM((2, RB, D), BF16),
            pltpu.SemaphoreType.DMA((12,)),
            pltpu.SemaphoreType.DMA((2,)),
            pltpu.SemaphoreType.DMA((2,)),
        ],
        compiler_params=pltpu.CompilerParams(
            dimension_semantics=("arbitrary",),
            vmem_limit_bytes=100 * 2 ** 20,
            disable_bounds_checks=True),
    )(*small, A_q[0], A_k[0], A_v[0], A_ssm_k, B_x[0], B_wqkv, B_wo)
    return out[None]
```

```python
import functools

import numpy as np
import jax
import jax.numpy as jnp
import jax.experimental.pallas as pl
import jax.experimental.pallas.tpu as pltpu

S = 2048
D = 1024
NH = 32
DH = 32
WIN = 8
DIL = 2
NSTEP = 8
RB = S // NSTEP
SUB = 128
HALO = 16
NBLK = 16
F32 = jnp.float32
BF16 = jnp.bfloat16
U32 = jnp.uint32
NT = (((1,), (1,)), ((), ()))
RATE, CRATE, QOFF, POFF, ASTEP, XLAT = 2.0, 2.5, 256, 384, 120, 192


def _constants():
    forder = np.concatenate([np.arange(0, 64, 2), np.arange(1, 64, 2)])
    theta = np.pi * (2 * forder + 1) / 256.0
    j = np.arange(128)
    ang = theta[:, None] * j[None, :]
    sgn = np.where(j % 2 == 0, 1.0, -1.0)[None, :]
    a_re, a_im = np.cos(ang), -np.sin(ang)
    b_re, b_im = a_re * sgn, a_im * sgn
    fwd = np.zeros((256, 128))
    for g in range(8):
        sl = slice(8 * g, 8 * g + 8)
        fwd[32 * g + 0:32 * g + 8] = a_re[sl]
        fwd[32 * g + 8:32 * g + 16] = a_im[sl]
        fwd[32 * g + 16:32 * g + 24] = b_re[sl]
        fwd[32 * g + 24:32 * g + 32] = b_im[sl]
    inv = np.zeros((2, 64, 128))
    s = np.arange(64)
    for p in range(2):
        a = (2 * s + p)[:, None] * theta[None, :]
        inv[p, :, 0::2] = np.cos(a) / 128.0
        inv[p, :, 1::2] = -np.sin(a) / 128.0
    perm = np.zeros((2, 128, 128))
    for jj in range(16):
        for r in range(8):
            hh = r % 4
            perm[0, 8 * jj + r, hh * 32 + 2 * jj + (r // 4)] = 1.0
            perm[1, 8 * jj + r, hh * 32 + 2 * jj + 1 - (r // 4)] = 1.0
    return (jnp.asarray(fwd, BF16), jnp.asarray(inv, BF16), jnp.asarray(perm, BF16))


def _lo(w):
    return pltpu.bitcast(w << 16, F32)


def _hi(w):
    return pltpu.bitcast(w & jnp.uint32(0xFFFF0000), F32)


def _ldb(ref32, *idx):
    return pltpu.bitcast(ref32[idx], BF16)


def _pk(a, b):
    return pltpu.pack_elementwise([a, b], packed_dtype=BF16)


def _kernel(sk_ref, d_ref, fw_ref, inv_ref, perm_ref,
            q_hbm, k_hbm, v_hbm, h_hbm, x_hbm, wqkv_hbm, wo_hbm, out_hbm,
            qin, kin, vin, hin, xin, wraw, woraw, wotmp, *rest):
    outa, outb, wsem, isem, osem = rest[-5:]
    step = pl.program_id(0)
    slot = step % 2

    def in_copies(st, sl, sems):
        c0 = pl.multiple_of(st * 128, 128)
        pairs = [(h_hbm.at[pl.ds(c0, 128), :], hin), (k_hbm.at[:, pl.ds(c0, 128)], kin),
                 (v_hbm.at[:, pl.ds(c0, 128)], vin),
                 (x_hbm.at[pl.ds(pl.multiple_of(st * RB, RB), RB), :], xin),
                 (q_hbm.at[:, pl.ds(c0, 128)], qin)]
        return [pltpu.make_async_copy(src, dst.at[sl], sem) for (src, dst), sem in zip(pairs, sems)]

    def out_copies(st, sl):
        return [
            pltpu.make_async_copy(
                outa.at[sl], out_hbm.at[:, pl.ds(pl.multiple_of(st * 128, 128), 128)], osem.at[sl]),
            pltpu.make_async_copy(
                outb.at[sl], out_hbm.at[pl.ds(pl.multiple_of(st * RB, RB), RB), pl.ds(D, D)],
                osem.at[sl])]

    nxt = in_copies(jnp.minimum(step + 1, NSTEP - 1), 1 - slot, [isem.at[1 - slot]] * 5)
    bufs = [r.at[slot] for r in (qin, kin, vin, hin, xin, outa, outb)]
    consts = (sk_ref, d_ref, fw_ref, inv_ref, perm_ref)

    @pl.when(step == 0)
    def _():
        dma = dict(zip("hkvxq", in_copies(0, 0, [wsem.at[j] for j in range(5)])))
        for j in range(4):
            rows = pl.ds(256 * j, 256)
            dma[j] = pltpu.make_async_copy(
                wqkv_hbm.at[rows, pl.ds(0, D)], wraw.at[0, rows, :], wsem.at[5 + j])
        for pp in (1, 2):
            dma["w%d" % pp] = pltpu.make_async_copy(
                wqkv_hbm.at[:, pl.ds(pp * D, D)], wraw.at[pp], wsem.at[8 + pp])
        for c in range(8):
            dma["o%d" % c] = pltpu.make_async_copy(
                wo_hbm.at[:, pl.ds(128 * c, 128)], woraw.at[c], wsem.at[11])
        for j, cp in enumerate(nxt):
            dma["n%d" % j] = cp
        _body(step, consts, bufs, (wraw, woraw, wotmp), rest[:-5], dma)

    @pl.when(step >= 2)
    def _():
        for cp in out_copies(step - 2, slot):
            cp.wait()

    @pl.when(step > 0)
    def _():
        for cp in in_copies(step, slot, [isem.at[slot]] * 5):
            cp.wait()
        for cp in nxt:
            cp.start()
        _body(step, consts, bufs, None, rest[:-5], None)

    for cp in out_copies(step, slot):
        cp.start()

    @pl.when(step == NSTEP - 1)
    def _():
        for cp in nxt + out_copies(step - 1, 1 - slot) + out_copies(step, slot):
            cp.wait()


def _body(step, consts, bufs, wsrc, scratch, dma):
    sk_ref, d_ref, fw_ref, inv_ref, perm_ref = consts
    q_ref, k_ref, v_ref, h_ref, x_ref, outa, outb = bufs
    wt0, wt1, wt2, wop, qs0, qs1, ks0, ks1, vs0, vs1, ob0, ob1, xb, ub, uf, hu, eo = scratch
    first = dma is not None
    al = slice(None)
    zero = step // NSTEP
    xz, ufz, eoz = (r.at[zero] for r in (xb, uf, eo))
    obz = [r.at[zero] for r in (ob0, ob1)]
    xb, ub, uf, eo = (r.at[0] for r in (xb, ub, uf, eo))
    ob = [r.at[0] for r in (ob0, ob1)]
    fw32, inv32 = fw_ref.bitcast(U32), inv_ref.bitcast(U32)
    wt32 = [r.bitcast(U32).at[zero] for r in (wt0, wt1, wt2)]
    wop32 = wop.at[zero]
    perm32 = perm_ref.bitcast(U32)
    k32 = k_ref.bitcast(U32)
    v32 = v_ref.bitcast(U32)
    q32 = q_ref.bitcast(U32)
    row8 = jax.lax.broadcasted_iota(jnp.int32, (8, 128), 0)
    sk = sk_ref[:, pl.ds(pl.multiple_of(step * 128, 128), 128)].astype(F32)
    taps = [jnp.broadcast_to(sk[j:j + 1, :], (8, 128)) for j in range(4)]
    dall = d_ref[...].astype(F32).reshape(8, 128)
    taps.append(jnp.broadcast_to(
        jnp.sum(jnp.where(row8 == step, dall, 0.0), axis=0, keepdims=True), (8, 128)))

    always = perm32[0, pl.ds(0, 8), :] != jnp.uint32(0x12345678)

    pend = []
    tnow = [0.0, 0.0, 1.0]

    cnt = [1]

    def fresh():
        cnt[0] += 1
        return zero * cnt[0]

    def due(val, ops, extra=0):
        tnow[1] += ops / tnow[2]
        pend.append((tnow[1] + extra, val))
        pend.sort(key=lambda e: e[0])

    def lhs(ref, r0, mod=8):
        tiles = [[ref[kt % mod, pl.ds(r0 // 2 + 8 * j, 8), :] for j in range(8)] for kt in range(8)]
        n = 0
        while pend and pend[0][0] < tnow[0] + 256:
            t, val = pend.pop(0)
            idx = max(int(t - tnow[0]), 0) // 16
            kt, j = 4 * (idx // 8) + n % 4, idx % 8
            tiles[kt][j] = jnp.where(always, tiles[kt][j], pltpu.bitcast(val, U32))
            n += 1
        return [pltpu.bitcast(jnp.concatenate(t, axis=0), BF16) for t in tiles]

    def a_fwd_h(m):
        r = jax.lax.dot_general(_ldb(fw32, al, al), h_ref[:, pl.ds(128 * m, 128)], NT,
                                preferred_element_type=F32)
        hu[0, m] = r

    def a_prep(i):
        tp = taps
        for r in range(8 * i, 8 * i + 8):
            w0 = k32[pl.ds(8 * r, 8), :]
            if r == 0:
                w1 = jnp.where(row8 < 1, jnp.uint32(0), pltpu.roll(w0, 1, 0))
                w2 = jnp.where(row8 < 2, jnp.uint32(0), pltpu.roll(w0, 2, 0))
            else:
                w1 = k32[pl.ds(8 * r - 1, 8), :]
                w2 = k32[pl.ds(8 * r - 2, 8), :]
            e0, o0, e1, o1, o2 = _lo(w0), _hi(w0), _lo(w1), _hi(w1), _hi(w2)
            kse = tp[0] * e0 + tp[1] * o1 + tp[2] * e1 + tp[3] * o2
            kso = tp[0] * o0 + tp[1] * e0 + tp[2] * o1 + tp[3] * e1
            wv = v32[pl.ds(8 * r, 8), :]
            ue = kse * _lo(wv)
            uo = kso * _hi(wv)
            pk = _pk(ue, uo)
            ub[pl.ds(8 * r, 8), :] = pk
            uf[0, pl.ds(8 * r, 8), :] = ue * taps[4]
            uf[1, pl.ds(8 * r, 8), :] = uo * taps[4]

    def a_fwd_u(i):
        r = jnp.dot(_ldb(fw32, al, al), _ldb(ub, pl.ds(64 * i, 64), al),
                    preferred_element_type=F32)
        hu[0, NBLK + i] = r

    conv_state = {}

    def a_conv(g, i):
        ys = []
        for ab in range(2):
            z = fresh()
            r_re, r_im = pl.ds(32 * g + 16 * ab, 8), pl.ds(32 * g + 16 * ab + 8, 8)
            for m in range(i + 1):
                hr, hi = hu[z, m, r_re, :], hu[z, m, r_im, :]
                ur, ui = hu[z, NBLK + i - m, r_re, :], hu[z, NBLK + i - m, r_im, :]
                yr = hr * ur if m == 0 else yr + hr * ur
                yi = hr * ui if m == 0 else yi + hr * ui
                yr, yi = yr - hi * ui, yi + hi * ur
            ys.append((yr, yi))
            if ab == 0:
                due(yr, 8 * i + 8)
                due(yi, 0)
        (ar, ai), (br, bi) = ys
        cur = (ar + br, ai + bi, ar - br, ai - bi)
        prev = conv_state.get("prev")
        if i == 0:
            res = cur
        elif g < 4:
            res = (cur[0] - prev[1], cur[1] + prev[0], cur[2] - prev[3], cur[3] + prev[2])
        else:
            res = (cur[0] + prev[1], cur[1] - prev[0], cur[2] + prev[3], cur[3] - prev[2])
        conv_state["prev"] = cur
        pe, po = _pk(res[0], res[1]), _pk(res[2], res[3])
        eo[i, 0, pl.ds(8 * g, 8), :] = pe
        eo[i, 1, pl.ds(8 * g, 8), :] = po
        due(pe, 8 * i + 18)
        due(po, 0)

    outa32 = outa.bitcast(U32)

    def a_inv(i):
        ye = jnp.dot(_ldb(inv32, 0), _ldb(eoz, i, 0), preferred_element_type=F32)
        yo = jnp.dot(_ldb(inv32, 1), _ldb(eoz, i, 1), preferred_element_type=F32)
        rows = pl.ds(64 * i, 64)
        wq = q32[rows, :]
        ae = (ye + ufz[0, rows, :]) * _lo(wq)
        ao = (yo + ufz[1, rows, :]) * _hi(wq)
        outa32[rows, :] = _pk(ae, ao)

    qs, ks, vs = (qs0, qs1), (ks0, ks1), (vs0, vs1)

    def b_qkv(sb, p, c2):
        r0 = sb * SUB
        acc = None
        xs = lhs(xz, r0)
        for kt in range(8):
            part = jax.lax.dot_general(
                xs[kt],
                _ldb(wt32[p], kt, pl.ds(c2 * 64, 64), al), NT,
                preferred_element_type=F32)
            acc = part if acc is None else acc + part
        if p == 0:
            qs[sb][0, c2] = acc
        else:
            dst = (ks, vs)[p - 1]
            dst[sb][0, c2, pl.ds(HALO, SUB), :] = acc
            if sb == 0:
                dst[1][0, c2, pl.ds(0, HALO), :] = acc[SUB - HALO:]

    cexp = float(DH ** -0.5 * np.log2(np.e))

    logits = {}
    outs = {}

    def b_rows(rt):
        return 32 * (rt // 4) + (0, 2, 1, 3)[rt % 4]

    def b_qk(rt):
        sb, r0 = rt // 16, b_rows(rt % 16)
        lg = [None] * WIN
        z = fresh()
        for c in range(8):
            qv = qs[sb][z, c, pl.ds(r0, 8, stride=4), :] * cexp
            for w in range(WIN):
                pr = qv * ks[sb][z, c, pl.ds(HALO - DIL * w + r0, 8, stride=4), :]
                lg[w] = pr if c == 0 else lg[w] + pr
        logits[rt] = [x + pltpu.roll(x, 64, 1) for x in lg]
        for x in logits[rt][3::4]:
            due(x, 72, XLAT)

    def b_q2(rt):
        sb, r0 = rt // 16, b_rows(rt % 16)
        lg = logits[rt]
        for w in range(WIN):
            acc = lg[w] + pltpu.roll(lg[w], 32, 1)
            if sb == 0 and r0 < DIL * w:
                acc = jnp.where(4 * row8 + (step * RB + r0) >= DIL * w, acc, -1e9)
            lg[w] = acc
            due(acc, 2, XLAT)

    def b_pv(rt):
        sb, r0 = rt // 16, b_rows(rt % 16)
        z = fresh()
        lg = logits.pop(rt)
        mx = functools.reduce(jnp.maximum, lg)
        ex = [jnp.exp2(l - mx) for l in lg]
        den = functools.reduce(lambda a, b: a + b, ex)
        rinv = pl.reciprocal(den, approx=True)
        rinv = rinv * (2.0 - den * rinv)
        o = [None] * 8
        for w in range(WIN):
            for c in range(8):
                pr = ex[w] * vs[sb][z, c, pl.ds(HALO - DIL * w + r0, 8, stride=4), :]
                o[c] = pr if w == 0 else o[c] + pr
        o = [x * rinv for x in o]
        outs[rt] = o
        if rt % 2 == 1:
            o0, o1 = outs.pop(rt - 1), outs.pop(rt)
            o = [_pk(o0[c], o1[c]) for c in range(8)]
            for c in range(8):
                ob[rt // 16][c, pl.ds(8 * (rt % 16 // 2), 8), :] = o[c]
        for x in o:
            due(x, 21)

    def b_out(sb, c):
        r0 = sb * SUB
        acc = None
        xs = lhs(obz[sb], 0)
        for kt in range(8):
            part = jnp.dot(xs[kt],
                           _ldb(wop32, c, pl.ds(64 * kt, 64), al),
                           preferred_element_type=F32)
            acc = part if acc is None else acc + part
        for j in range(SUB // 32):
            outb[pl.ds(r0 + 32 * j, 32), pl.ds(128 * c, 128)] = pltpu.bitcast(_pk(
                acc[32 * j:32 * j + 16], acc[32 * j + 16:32 * j + 32]), BF16)

    def b_x():
        for kt in range(8):
            xb[kt] = pltpu.bitcast(x_ref[:, pl.ds(128 * kt, 128)], U32)

    def w_perm(p, kt):
        low = jax.lax.broadcasted_iota(jnp.int32, (16, 8, 128), 1) < 4
        sel = lhs(perm32, 0, 2)
        tr = [jax.lax.dot_general(
            sel[t], wsrc[0][p, pl.ds(128 * kt, 128), pl.ds(128 * t, 128)], NT,
            preferred_element_type=F32).reshape(16, 8, 128) for t in range(8)]
        for h4 in range(2):
            ev = [jnp.where(low, tr[t], tr[t + 1]) for t in (4 * h4, 4 * h4 + 2)]
            od = [pltpu.roll(jnp.where(low, tr[t + 1], tr[t]), 4, 1) for t in (4 * h4, 4 * h4 + 2)]
            for jj in range(16):
                for par, src in ((0, ev), (1, od)):
                    blk = jnp.concatenate([src[0][jj], src[1][jj]], axis=0)
                    (wt0, wt1, wt2)[p][0, kt, pl.ds((2 * jj + par) * 32 + h4 * 16, 16), :] = (
                        blk.astype(BF16))

    def wo_perm(c):
        wo32, tmp = wsrc[1].bitcast(U32), wsrc[2]
        for g in range(16):
            tmp[c, pl.ds(36 * g, 32), :] = wo32[c, pl.ds(32 * g, 32), :]
        for dd in range(16):
            for h4 in range(2):
                a = tmp[c, pl.ds(h4 * 288 + dd, 8, stride=36), :]
                b = tmp[c, pl.ds(h4 * 288 + 16 + dd, 8, stride=36), :]
                wop[0, c, pl.ds((2 * dd) * 16 + h4 * 8, 8), :] = (
                    (a & jnp.uint32(0xFFFF)) | (b << 16))
                hi = (a >> 16) | (b & jnp.uint32(0xFFFF0000))
                wop[0, c, pl.ds((2 * dd + 1) * 16 + h4 * 8, 8), :] = hi
                due(hi, 8, 256)

    def sync(wait, start):
        for key in wait:
            dma[key].wait()
        for key in start:
            dma[key].start()

    P = functools.partial
    qkv = lambda sb, p, cs=range(8): [(P(b_qkv, sb, p, c), 256) for c in cs]
    fwd_h = [(P(a_fwd_h, i), 64) for i in range(NBLK)]
    fwd_u = [(P(a_fwd_u, i), 64) for i in range(NBLK)]
    tail = ([(P(a_inv, i), 32) for i in range(NBLK)]
            + [(P(b_out, sb, c), 256) for sb in range(2) for c in range(8)])

    def conv(t, rate):
        for g in range(8):
            for i in range(NBLK):
                vpu.append((t, rate, P(a_conv, g, i)))
                t += (16 * i + 26) / rate

    def att(fn, sb, t, dt):
        vpu.extend((t + dt * j, RATE, P(fn, 16 * sb + j)) for j in range(16))

    if first:
        ks0[0, :, pl.ds(0, HALO), :] = jnp.zeros((8, HALO, 128), F32)
        vs0[0, :, pl.ds(0, HALO), :] = jnp.zeros((8, HALO, 128), F32)
        wos = ["o%d" % c for c in range(8)]
        perm = lambda p, kts=range(8): [(P(w_perm, p, kt), 256) for kt in kts]
        sy = lambda wait, start=(): [(P(sync, wait, start), 0)]
        mxu = (sy([], [0, 1]) + sy([0], [2]) + perm(0, (0, 1)) + sy([1], [3, "x"])
               + perm(0, (2, 3)) + sy([2], "h") + perm(0, (4, 5)) + sy([3, "x"], ["k", "v", "w1"])
               + [(b_x, 0)] + perm(0, (6, 7)) + qkv(0, 0) + sy([], ["w2"]) + qkv(1, 0, range(4))
               + sy("hkv") + fwd_h + qkv(1, 0, range(4, 8)) + fwd_u
               + sy(["w1"], ["q"] + wos) + perm(1) + qkv(0, 1)
               + sy(["w2"], ["n%d" % j for j in range(5)]) + perm(2) + qkv(1, 1)
               + qkv(0, 2, range(4)) + sy(["q"] + wos) + qkv(0, 2, range(4, 8)) + qkv(1, 2) + tail)
        vpu = [(6144 + 64 * i, 1, P(a_prep, i)) for i in range(NBLK)]
        conv(8192.0 + POFF, 2.3)
        for sb, t in ((0, 15000), (1, 16896)):
            att(b_qk, sb, t, ASTEP)
            att(b_q2, sb, t + 260, ASTEP)
            att(b_pv, sb, 18432 + POFF + 2048 * sb, ASTEP)
        vpu += [(17408 + 256 * c, 1, P(wo_perm, c)) for c in range(8)]
    else:
        mxu = ([(b_x, 0)] + fwd_h + qkv(0, 2, range(2)) + fwd_u + qkv(0, 2, range(2, 8))
               + qkv(0, 0) + qkv(0, 1) + qkv(1, 0) + qkv(1, 1) + qkv(1, 2) + tail)
        vpu = [(512 + 64 * i, 1, P(a_prep, i)) for i in range(NBLK)]
        conv(2560.0 + POFF, CRATE)
        att(b_qk, 0, 8192 + QOFF, 224)
        att(b_q2, 0, 8192 + QOFF + 230, 224)
        att(b_pv, 0, 8192 + QOFF + 560, 224)
        att(b_qk, 1, 12288 + QOFF, ASTEP)
        att(b_q2, 1, 12288 + QOFF + 260, ASTEP)
        att(b_pv, 1, 14336 + POFF, ASTEP)
    vpu.sort(key=lambda e: e[0])
    for fn, cyc in mxu:
        while vpu and vpu[0][0] < tnow[0] + cyc:
            tnow[1], tnow[2], unit = vpu.pop(0)
            unit()
        fn()
        tnow[0] += cyc
    assert not vpu
    ks0[0, :, pl.ds(0, HALO), :] = ks1[0, :, pl.ds(SUB, HALO), :]
    vs0[0, :, pl.ds(0, HALO), :] = vs1[0, :, pl.ds(SUB, HALO), :]


@jax.jit
def pallas_concat_heads__ssm_conv_h3__sliding_local_dilated__prompt_kernel(
    A_q: jax.Array,
    A_k: jax.Array,
    A_v: jax.Array,
    A_shift_k: jax.Array,
    A_ssm_k: jax.Array,
    A_ssm_D: jax.Array,
    B_x: jax.Array,
    B_wqkv: jax.Array,
    B_wo: jax.Array,
):
    fw, inv, perm = _constants()
    small = (A_shift_k.T, A_ssm_D, fw, inv, perm)
    full = lambda a: pl.BlockSpec(a.shape, lambda s: (0,) * a.ndim)
    out = pl.pallas_call(
        _kernel,
        grid=(NSTEP,),
        in_specs=[full(a) for a in small] + [pl.BlockSpec(memory_space=pl.ANY)] * 7,
        out_specs=pl.BlockSpec(memory_space=pl.ANY),
        out_shape=jax.ShapeDtypeStruct((S, 2 * D), BF16),
        scratch_shapes=[
            pltpu.VMEM((2, S, 128), BF16),
            pltpu.VMEM((2, S, 128), BF16),
            pltpu.VMEM((2, S, 128), BF16),
            pltpu.VMEM((2, 128, S), BF16),
            pltpu.VMEM((2, RB, D), BF16),
            pltpu.VMEM((3, D, D), BF16),
            pltpu.VMEM((8, D, 128), BF16),
            pltpu.VMEM((8, 576, 128), U32),
            pltpu.VMEM((1, 8, D, 128), BF16),
            pltpu.VMEM((1, 8, D, 128), BF16),
            pltpu.VMEM((1, 8, D, 128), BF16),
            pltpu.VMEM((1, 8, D // 2, 128), U32),
            pltpu.VMEM((1, 8, SUB, 128), F32),
            pltpu.VMEM((1, 8, SUB, 128), F32),
            pltpu.VMEM((1, 8, HALO + SUB, 128), F32),
            pltpu.VMEM((1, 8, HALO + SUB, 128), F32),
            pltpu.VMEM((1, 8, HALO + SUB, 128), F32),
            pltpu.VMEM((1, 8, HALO + SUB, 128), F32),
            pltpu.VMEM((1, 8, SUB // 2, 128), U32),
            pltpu.VMEM((1, 8, SUB // 2, 128), U32),
            pltpu.VMEM((1, 8, RB // 2, 128), U32),
            pltpu.VMEM((1, S // 2, 128), U32),
            pltpu.VMEM((1, 2, S // 2, 128), F32),
            pltpu.VMEM((1, 2 * NBLK, 256, 128), F32),
            pltpu.VMEM((1, NBLK, 2, 64, 128), U32),
            pltpu.VMEM((2, S, 128), BF16),
            pltpu.VMEM((2, RB, D), BF16),
            pltpu.SemaphoreType.DMA((12,)),
            pltpu.SemaphoreType.DMA((2,)),
            pltpu.SemaphoreType.DMA((2,)),
        ],
        compiler_params=pltpu.CompilerParams(
            dimension_semantics=("arbitrary",),
            vmem_limit_bytes=100 * 2 ** 20,
            disable_bounds_checks=True),
    )(*small, A_q[0], A_k[0], A_v[0], A_ssm_k, B_x[0], B_wqkv, B_wo)
    return out[None]
```

```python
import functools

import numpy as np
import jax
import jax.numpy as jnp
import jax.experimental.pallas as pl
import jax.experimental.pallas.tpu as pltpu

S = 2048
D = 1024
NH = 32
DH = 32
WIN = 8
DIL = 2
NSTEP = 8
RB = S // NSTEP
SUB = 128
HALO = 16
NBLK = 16
F32 = jnp.float32
BF16 = jnp.bfloat16
U32 = jnp.uint32
NT = (((1,), (1,)), ((), ()))
RATE, CRATE, QOFF, POFF, ASTEP, XLAT = 2.4, 2.5, 384, 384, 120, 192


def _constants():
    forder = np.concatenate([np.arange(0, 64, 2), np.arange(1, 64, 2)])
    theta = np.pi * (2 * forder + 1) / 256.0
    j = np.arange(128)
    ang = theta[:, None] * j[None, :]
    sgn = np.where(j % 2 == 0, 1.0, -1.0)[None, :]
    a_re, a_im = np.cos(ang), -np.sin(ang)
    b_re, b_im = a_re * sgn, a_im * sgn
    fwd = np.zeros((256, 128))
    for g in range(8):
        sl = slice(8 * g, 8 * g + 8)
        fwd[32 * g + 0:32 * g + 8] = a_re[sl]
        fwd[32 * g + 8:32 * g + 16] = a_im[sl]
        fwd[32 * g + 16:32 * g + 24] = b_re[sl]
        fwd[32 * g + 24:32 * g + 32] = b_im[sl]
    inv = np.zeros((2, 64, 128))
    s = np.arange(64)
    for p in range(2):
        a = (2 * s + p)[:, None] * theta[None, :]
        inv[p, :, 0::2] = np.cos(a) / 128.0
        inv[p, :, 1::2] = -np.sin(a) / 128.0
    perm = np.zeros((2, 128, 128))
    for jj in range(16):
        for r in range(8):
            hh = r % 4
            perm[0, 8 * jj + r, hh * 32 + 2 * jj + (r // 4)] = 1.0
            perm[1, 8 * jj + r, hh * 32 + 2 * jj + 1 - (r // 4)] = 1.0
    return (jnp.asarray(fwd, BF16), jnp.asarray(inv, BF16), jnp.asarray(perm, BF16))


def _lo(w):
    return pltpu.bitcast(w << 16, F32)


def _hi(w):
    return pltpu.bitcast(w & jnp.uint32(0xFFFF0000), F32)


def _ldb(ref32, *idx):
    return pltpu.bitcast(ref32[idx], BF16)


def _pk(a, b):
    return pltpu.pack_elementwise([a, b], packed_dtype=BF16)


def _kernel(sk_ref, d_ref, fw_ref, inv_ref, perm_ref,
            q_hbm, k_hbm, v_hbm, h_hbm, x_hbm, wqkv_hbm, wo_hbm, out_hbm,
            qin, kin, vin, hin, xin, wraw, woraw, wotmp, *rest):
    outa, outb, wsem, isem, osem = rest[-5:]
    step = pl.program_id(0)
    slot = step % 2

    def in_copies(st, sl, sems):
        c0 = pl.multiple_of(st * 128, 128)
        pairs = [(h_hbm.at[pl.ds(c0, 128), :], hin), (k_hbm.at[:, pl.ds(c0, 128)], kin),
                 (v_hbm.at[:, pl.ds(c0, 128)], vin),
                 (x_hbm.at[pl.ds(pl.multiple_of(st * RB, RB), RB), :], xin),
                 (q_hbm.at[:, pl.ds(c0, 128)], qin)]
        return [pltpu.make_async_copy(src, dst.at[sl], sem) for (src, dst), sem in zip(pairs, sems)]

    def out_copies(st, sl):
        return [
            pltpu.make_async_copy(
                outa.at[sl], out_hbm.at[:, pl.ds(pl.multiple_of(st * 128, 128), 128)], osem.at[sl]),
        ] + [pltpu.make_async_copy(
            outb.at[sl, pl.ds(sb * SUB, SUB), :],
            out_hbm.at[pl.ds(pl.multiple_of(st * RB + sb * SUB, SUB), SUB), pl.ds(D, D)],
            osem.at[sl]) for sb in range(2)]

    outs = out_copies(step, slot)
    nxt = in_copies(jnp.minimum(step + 1, NSTEP - 1), 1 - slot, [isem.at[1 - slot]] * 5)
    bufs = [r.at[slot] for r in (qin, kin, vin, hin, xin, outa, outb)]
    consts = (sk_ref, d_ref, fw_ref, inv_ref, perm_ref)

    @pl.when(step == 0)
    def _():
        dma = dict(zip("hkvxq", in_copies(0, 0, [wsem.at[j] for j in range(5)])))
        for j in range(4):
            rows = pl.ds(256 * j, 256)
            dma[j] = pltpu.make_async_copy(
                wqkv_hbm.at[rows, pl.ds(0, D)], wraw.at[0, rows, :], wsem.at[5 + j])
        for pp in (1, 2):
            dma["w%d" % pp] = pltpu.make_async_copy(
                wqkv_hbm.at[:, pl.ds(pp * D, D)], wraw.at[pp], wsem.at[8 + pp])
        for c in range(8):
            dma["o%d" % c] = pltpu.make_async_copy(
                wo_hbm.at[:, pl.ds(128 * c, 128)], woraw.at[c], wsem.at[11])
        for j, cp in enumerate(nxt):
            dma["n%d" % j] = cp
        _body(step, consts, bufs, (wraw, woraw, wotmp), rest[:-5], dma, outs)

    @pl.when(step >= 2)
    def _():
        for cp in out_copies(step - 2, slot):
            cp.wait()

    @pl.when(step > 0)
    def _():
        for cp in in_copies(step, slot, [isem.at[slot]] * 5):
            cp.wait()
        for cp in nxt:
            cp.start()
        _body(step, consts, bufs, None, rest[:-5], None, outs)

    @pl.when(step == NSTEP - 1)
    def _():
        for cp in nxt + out_copies(step - 1, 1 - slot) + outs:
            cp.wait()


def _body(step, consts, bufs, wsrc, scratch, dma, out_dma):
    sk_ref, d_ref, fw_ref, inv_ref, perm_ref = consts
    q_ref, k_ref, v_ref, h_ref, x_ref, outa, outb = bufs
    wt0, wt1, wt2, wop, qs0, qs1, ks0, ks1, vs0, vs1, ob0, ob1, xb, ub, uf, hu, eo = scratch
    first = dma is not None
    al = slice(None)
    zero = step // NSTEP
    xz, ufz, eoz = (r.at[zero] for r in (xb, uf, eo))
    obz = [r.at[zero] for r in (ob0, ob1)]
    xb, ub, uf, eo = (r.at[0] for r in (xb, ub, uf, eo))
    ob = [r.at[0] for r in (ob0, ob1)]
    fw32, inv32 = fw_ref.bitcast(U32), inv_ref.bitcast(U32)
    wt32 = [r.bitcast(U32).at[zero] for r in (wt0, wt1, wt2)]
    wop32 = wop.at[zero]
    perm32 = perm_ref.bitcast(U32)
    k32 = k_ref.bitcast(U32)
    v32 = v_ref.bitcast(U32)
    q32 = q_ref.bitcast(U32)
    row8 = jax.lax.broadcasted_iota(jnp.int32, (8, 128), 0)
    sk = sk_ref[:, pl.ds(pl.multiple_of(step * 128, 128), 128)].astype(F32)
    taps = [jnp.broadcast_to(sk[j:j + 1, :], (8, 128)) for j in range(4)]
    dall = d_ref[...].astype(F32).reshape(8, 128)
    taps.append(jnp.broadcast_to(
        jnp.sum(jnp.where(row8 == step, dall, 0.0), axis=0, keepdims=True), (8, 128)))

    always = perm32[0, pl.ds(0, 8), :] != jnp.uint32(0x12345678)

    pend = []
    tnow = [0.0, 0.0, 1.0]

    cnt = [1]

    def fresh():
        cnt[0] += 1
        return zero * cnt[0]

    def due(val, ops, extra=0):
        tnow[1] += ops / tnow[2]
        pend.append((tnow[1] + extra, val))
        pend.sort(key=lambda e: e[0])

    def lhs(ref, r0, mod=8):
        tiles = [[ref[kt % mod, pl.ds(r0 // 2 + 8 * j, 8), :] for j in range(8)] for kt in range(8)]
        n = 0
        while pend and pend[0][0] < tnow[0] + 256:
            t, val = pend.pop(0)
            idx = max(int(t - tnow[0]), 0) // 16
            kt, j = 4 * (idx // 8) + n % 4, idx % 8
            tiles[kt][j] = jnp.where(always, tiles[kt][j], pltpu.bitcast(val, U32))
            n += 1
        return [pltpu.bitcast(jnp.concatenate(t, axis=0), BF16) for t in tiles]

    def a_fwd_h(m):
        r = jax.lax.dot_general(_ldb(fw32, al, al), h_ref[:, pl.ds(128 * m, 128)], NT,
                                preferred_element_type=F32)
        hu[0, m] = r

    def a_prep(i):
        tp = taps
        for r in range(8 * i, 8 * i + 8):
            w0 = k32[pl.ds(8 * r, 8), :]
            if r == 0:
                w1 = jnp.where(row8 < 1, jnp.uint32(0), pltpu.roll(w0, 1, 0))
                w2 = jnp.where(row8 < 2, jnp.uint32(0), pltpu.roll(w0, 2, 0))
            else:
                w1 = k32[pl.ds(8 * r - 1, 8), :]
                w2 = k32[pl.ds(8 * r - 2, 8), :]
            e0, o0, e1, o1, o2 = _lo(w0), _hi(w0), _lo(w1), _hi(w1), _hi(w2)
            kse = tp[0] * e0 + tp[1] * o1 + tp[2] * e1 + tp[3] * o2
            kso = tp[0] * o0 + tp[1] * e0 + tp[2] * o1 + tp[3] * e1
            wv = v32[pl.ds(8 * r, 8), :]
            ue = kse * _lo(wv)
            uo = kso * _hi(wv)
            pk = _pk(ue, uo)
            ub[pl.ds(8 * r, 8), :] = pk
            uf[0, pl.ds(8 * r, 8), :] = ue * taps[4]
            uf[1, pl.ds(8 * r, 8), :] = uo * taps[4]

    def a_fwd_u(i):
        r = jnp.dot(_ldb(fw32, al, al), _ldb(ub, pl.ds(64 * i, 64), al),
                    preferred_element_type=F32)
        hu[0, NBLK + i] = r

    conv_state = {}

    def a_conv(g, i):
        ys = []
        for ab in range(2):
            z = fresh()
            r_re, r_im = pl.ds(32 * g + 16 * ab, 8), pl.ds(32 * g + 16 * ab + 8, 8)
            for m in range(i + 1):
                hr, hi = hu[z, m, r_re, :], hu[z, m, r_im, :]
                ur, ui = hu[z, NBLK + i - m, r_re, :], hu[z, NBLK + i - m, r_im, :]
                yr = hr * ur if m == 0 else yr + hr * ur
                yi = hr * ui if m == 0 else yi + hr * ui
                yr, yi = yr - hi * ui, yi + hi * ur
            ys.append((yr, yi))
            if ab == 0:
                due(yr, 8 * i + 8)
                due(yi, 0)
        (ar, ai), (br, bi) = ys
        cur = (ar + br, ai + bi, ar - br, ai - bi)
        prev = conv_state.get("prev")
        if i == 0:
            res = cur
        elif g < 4:
            res = (cur[0] - prev[1], cur[1] + prev[0], cur[2] - prev[3], cur[3] + prev[2])
        else:
            res = (cur[0] + prev[1], cur[1] - prev[0], cur[2] + prev[3], cur[3] - prev[2])
        conv_state["prev"] = cur
        pe, po = _pk(res[0], res[1]), _pk(res[2], res[3])
        eo[i, 0, pl.ds(8 * g, 8), :] = pe
        eo[i, 1, pl.ds(8 * g, 8), :] = po
        due(pe, 8 * i + 18)
        due(po, 0)

    outa32 = outa.bitcast(U32)

    def a_inv(i):
        ye = jnp.dot(_ldb(inv32, 0), _ldb(eoz, i, 0), preferred_element_type=F32)
        yo = jnp.dot(_ldb(inv32, 1), _ldb(eoz, i, 1), preferred_element_type=F32)
        rows = pl.ds(64 * i, 64)
        wq = q32[rows, :]
        ae = (ye + ufz[0, rows, :]) * _lo(wq)
        ao = (yo + ufz[1, rows, :]) * _hi(wq)
        outa32[rows, :] = _pk(ae, ao)

    qs, ks, vs = (qs0, qs1), (ks0, ks1), (vs0, vs1)

    def b_qkv(sb, p, c2):
        r0 = sb * SUB
        acc = None
        xs = lhs(xz, r0)
        for kt in range(8):
            part = jax.lax.dot_general(
                xs[kt],
                _ldb(wt32[p], kt, pl.ds(c2 * 64, 64), al), NT,
                preferred_element_type=F32)
            acc = part if acc is None else acc + part
        if p == 0:
            qs[sb][0, c2] = acc
        else:
            dst = (ks, vs)[p - 1]
            dst[sb][0, c2, pl.ds(HALO, SUB), :] = acc
            if sb == 0:
                dst[1][0, c2, pl.ds(0, HALO), :] = acc[SUB - HALO:]

    cexp = float(DH ** -0.5 * np.log2(np.e))

    logits = {}
    outs = {}

    def b_rows(rt):
        return 32 * (rt // 4) + (0, 2, 1, 3)[rt % 4]

    def b_qk(rt):
        sb, r0 = rt // 16, b_rows(rt % 16)
        lg = [None] * WIN
        z = fresh()
        for c in range(8):
            qv = qs[sb][z, c, pl.ds(r0, 8, stride=4), :] * cexp
            for w in range(WIN):
                pr = qv * ks[sb][z, c, pl.ds(HALO - DIL * w + r0, 8, stride=4), :]
                lg[w] = pr if c == 0 else lg[w] + pr
        logits[rt] = [x + pltpu.roll(x, 64, 1) for x in lg]
        for x in logits[rt][3::4]:
            due(x, 72, XLAT)

    def b_q2(rt):
        sb, r0 = rt // 16, b_rows(rt % 16)
        lg = logits[rt]
        for w in range(WIN):
            acc = lg[w] + pltpu.roll(lg[w], 32, 1)
            if sb == 0 and r0 < DIL * w:
                acc = jnp.where(4 * row8 + (step * RB + r0) >= DIL * w, acc, -1e9)
            lg[w] = acc
            due(acc, 2, XLAT)

    def b_pv(rt):
        sb, r0 = rt // 16, b_rows(rt % 16)
        z = fresh()
        lg = logits.pop(rt)
        mx = functools.reduce(jnp.maximum, lg)
        ex = [jnp.exp2(l - mx) for l in lg]
        den = functools.reduce(lambda a, b: a + b, ex)
        rinv = pl.reciprocal(den, approx=True)
        rinv = rinv * (2.0 - den * rinv)
        o = [None] * 8
        for w in range(WIN):
            for c in range(8):
                pr = ex[w] * vs[sb][z, c, pl.ds(HALO - DIL * w + r0, 8, stride=4), :]
                o[c] = pr if w == 0 else o[c] + pr
        o = [x * rinv for x in o]
        outs[rt] = o
        if rt % 2 == 1:
            o0, o1 = outs.pop(rt - 1), outs.pop(rt)
            o = [_pk(o0[c], o1[c]) for c in range(8)]
            for c in range(8):
                ob[rt // 16][c, pl.ds(8 * (rt % 16 // 2), 8), :] = o[c]
        for x in o:
            due(x, 21)

    def b_out(sb, c):
        r0 = sb * SUB
        acc = None
        xs = lhs(obz[sb], 0)
        for kt in range(8):
            part = jnp.dot(xs[kt],
                           _ldb(wop32, c, pl.ds(64 * kt, 64), al),
                           preferred_element_type=F32)
            acc = part if acc is None else acc + part
        for j in range(SUB // 32):
            outb[pl.ds(r0 + 32 * j, 32), pl.ds(128 * c, 128)] = pltpu.bitcast(_pk(
                acc[32 * j:32 * j + 16], acc[32 * j + 16:32 * j + 32]), BF16)

    def b_x():
        for kt in range(8):
            xb[kt] = pltpu.bitcast(x_ref[:, pl.ds(128 * kt, 128)], U32)

    def w_perm(p, kt):
        low = jax.lax.broadcasted_iota(jnp.int32, (16, 8, 128), 1) < 4
        sel = lhs(perm32, 0, 2)
        tr = [jax.lax.dot_general(
            sel[t], wsrc[0][p, pl.ds(128 * kt, 128), pl.ds(128 * t, 128)], NT,
            preferred_element_type=F32).reshape(16, 8, 128) for t in range(8)]
        for h4 in range(2):
            ev = [jnp.where(low, tr[t], tr[t + 1]) for t in (4 * h4, 4 * h4 + 2)]
            od = [pltpu.roll(jnp.where(low, tr[t + 1], tr[t]), 4, 1) for t in (4 * h4, 4 * h4 + 2)]
            for jj in range(16):
                for par, src in ((0, ev), (1, od)):
                    blk = jnp.concatenate([src[0][jj], src[1][jj]], axis=0)
                    (wt0, wt1, wt2)[p][0, kt, pl.ds((2 * jj + par) * 32 + h4 * 16, 16), :] = (
                        blk.astype(BF16))

    def wo_perm(c):
        wo32, tmp = wsrc[1].bitcast(U32), wsrc[2]
        for g in range(16):
            tmp[c, pl.ds(36 * g, 32), :] = wo32[c, pl.ds(32 * g, 32), :]
        for dd in range(16):
            for h4 in range(2):
                a = tmp[c, pl.ds(h4 * 288 + dd, 8, stride=36), :]
                b = tmp[c, pl.ds(h4 * 288 + 16 + dd, 8, stride=36), :]
                wop[0, c, pl.ds((2 * dd) * 16 + h4 * 8, 8), :] = (
                    (a & jnp.uint32(0xFFFF)) | (b << 16))
                hi = (a >> 16) | (b & jnp.uint32(0xFFFF0000))
                wop[0, c, pl.ds((2 * dd + 1) * 16 + h4 * 8, 8), :] = hi
                due(hi, 8, 256)

    def sync(wait, start):
        for key in wait:
            dma[key].wait()
        for key in start:
            dma[key].start()

    P = functools.partial
    qkv = lambda sb, p, cs=range(8): [(P(b_qkv, sb, p, c), 256) for c in cs]
    fwd_h = [(P(a_fwd_h, i), 64) for i in range(NBLK)]
    fwd_u = [(P(a_fwd_u, i), 64) for i in range(NBLK)]
    tail = ([(P(a_inv, i), 32) for i in range(NBLK)]
            + [(P(b_out, sb, c), 256) for sb in range(2) for c in range(8)])
    tail.insert(NBLK + 10, (lambda: [cp.start() for cp in out_dma[:2]], 0))
    tail.append((out_dma[2].start, 0))

    def conv(t, rate):
        for g in range(8):
            for i in range(NBLK):
                vpu.append((t, rate, P(a_conv, g, i)))
                t += (16 * i + 26) / rate

    def att(fn, sb, t, dt):
        vpu.extend((t + dt * j, RATE, P(fn, 16 * sb + j)) for j in range(16))

    if first:
        ks0[0, :, pl.ds(0, HALO), :] = jnp.zeros((8, HALO, 128), F32)
        vs0[0, :, pl.ds(0, HALO), :] = jnp.zeros((8, HALO, 128), F32)
        wos = ["o%d" % c for c in range(8)]
        perm = lambda p, kts=range(8): [(P(w_perm, p, kt), 256) for kt in kts]
        sy = lambda wait, start=(): [(P(sync, wait, start), 0)]
        mxu = (sy([], [0, 1]) + sy([0], [2]) + perm(0, (0, 1)) + sy([1], [3, "x"])
               + perm(0, (2, 3)) + sy([2], "h") + perm(0, (4, 5)) + sy([3, "x"], ["k", "v", "w1"])
               + [(b_x, 0)] + perm(0, (6, 7)) + qkv(0, 0) + sy([], ["w2"]) + qkv(1, 0, range(4))
               + sy("hkv") + fwd_h + qkv(1, 0, range(4, 8)) + fwd_u
               + sy(["w1"], ["q"] + wos) + perm(1) + qkv(0, 1)
               + sy(["w2"], ["n%d" % j for j in range(5)]) + perm(2) + qkv(1, 1)
               + qkv(0, 2, range(4)) + sy(["q"] + wos) + qkv(0, 2, range(4, 8)) + qkv(1, 2) + tail)
        vpu = [(6144 + 64 * i, 1, P(a_prep, i)) for i in range(NBLK)]
        conv(8192.0 + POFF, 2.3)
        for sb, t in ((0, 15000), (1, 16896)):
            att(b_qk, sb, t, ASTEP)
            att(b_q2, sb, t + 260, ASTEP)
            att(b_pv, sb, 18432 + POFF + 2048 * sb, ASTEP)
        vpu += [(17408 + 256 * c, 1, P(wo_perm, c)) for c in range(8)]
    else:
        mxu = ([(b_x, 0)] + fwd_h[:4] + qkv(0, 2, range(1)) + [e for p in zip(fwd_u, fwd_h[4:]) for e in p]
               + fwd_u[NBLK - 4:] + qkv(0, 2, range(1, 2)) + qkv(0, 2, range(2, 8))
               + qkv(0, 0) + qkv(0, 1) + qkv(1, 0) + qkv(1, 1) + qkv(1, 2) + tail)
        vpu = [(100 * i, 1, P(a_prep, i)) for i in range(NBLK)]
        conv(2560.0 + POFF, CRATE)
        att(b_qk, 0, 8192 + QOFF, 224)
        att(b_q2, 0, 8192 + QOFF + 230, 224)
        att(b_pv, 0, 8192 + QOFF + 560, 224)
        att(b_qk, 1, 12288 + QOFF, ASTEP)
        att(b_q2, 1, 12288 + QOFF + 260, ASTEP)
        att(b_pv, 1, 14336 + POFF, ASTEP)
    vpu.sort(key=lambda e: e[0])
    for fn, cyc in mxu:
        while vpu and vpu[0][0] < tnow[0] + cyc:
            tnow[1], tnow[2], unit = vpu.pop(0)
            unit()
        fn()
        tnow[0] += cyc
    assert not vpu
    ks0[0, :, pl.ds(0, HALO), :] = ks1[0, :, pl.ds(SUB, HALO), :]
    vs0[0, :, pl.ds(0, HALO), :] = vs1[0, :, pl.ds(SUB, HALO), :]


@jax.jit
def pallas_concat_heads__ssm_conv_h3__sliding_local_dilated__prompt_kernel(
    A_q: jax.Array,
    A_k: jax.Array,
    A_v: jax.Array,
    A_shift_k: jax.Array,
    A_ssm_k: jax.Array,
    A_ssm_D: jax.Array,
    B_x: jax.Array,
    B_wqkv: jax.Array,
    B_wo: jax.Array,
):
    fw, inv, perm = _constants()
    small = (A_shift_k.T, A_ssm_D, fw, inv, perm)
    full = lambda a: pl.BlockSpec(a.shape, lambda s: (0,) * a.ndim)
    out = pl.pallas_call(
        _kernel,
        grid=(NSTEP,),
        in_specs=[full(a) for a in small] + [pl.BlockSpec(memory_space=pl.ANY)] * 7,
        out_specs=pl.BlockSpec(memory_space=pl.ANY),
        out_shape=jax.ShapeDtypeStruct((S, 2 * D), BF16),
        scratch_shapes=[
            pltpu.VMEM((2, S, 128), BF16),
            pltpu.VMEM((2, S, 128), BF16),
            pltpu.VMEM((2, S, 128), BF16),
            pltpu.VMEM((2, 128, S), BF16),
            pltpu.VMEM((2, RB, D), BF16),
            pltpu.VMEM((3, D, D), BF16),
            pltpu.VMEM((8, D, 128), BF16),
            pltpu.VMEM((8, 576, 128), U32),
            pltpu.VMEM((1, 8, D, 128), BF16),
            pltpu.VMEM((1, 8, D, 128), BF16),
            pltpu.VMEM((1, 8, D, 128), BF16),
            pltpu.VMEM((1, 8, D // 2, 128), U32),
            pltpu.VMEM((1, 8, SUB, 128), F32),
            pltpu.VMEM((1, 8, SUB, 128), F32),
            pltpu.VMEM((1, 8, HALO + SUB, 128), F32),
            pltpu.VMEM((1, 8, HALO + SUB, 128), F32),
            pltpu.VMEM((1, 8, HALO + SUB, 128), F32),
            pltpu.VMEM((1, 8, HALO + SUB, 128), F32),
            pltpu.VMEM((1, 8, SUB // 2, 128), U32),
            pltpu.VMEM((1, 8, SUB // 2, 128), U32),
            pltpu.VMEM((1, 8, RB // 2, 128), U32),
            pltpu.VMEM((1, S // 2, 128), U32),
            pltpu.VMEM((1, 2, S // 2, 128), F32),
            pltpu.VMEM((1, 2 * NBLK, 256, 128), F32),
            pltpu.VMEM((1, NBLK, 2, 64, 128), U32),
            pltpu.VMEM((2, S, 128), BF16),
            pltpu.VMEM((2, RB, D), BF16),
            pltpu.SemaphoreType.DMA((12,)),
            pltpu.SemaphoreType.DMA((2,)),
            pltpu.SemaphoreType.DMA((2,)),
        ],
        compiler_params=pltpu.CompilerParams(
            dimension_semantics=("arbitrary",),
            vmem_limit_bytes=100 * 2 ** 20,
            disable_bounds_checks=True),
    )(*small, A_q[0], A_k[0], A_v[0], A_ssm_k, B_x[0], B_wqkv, B_wo)
    return out[None]
```
